```python
import jax
import jax.numpy as jnp

def _softmax(x, axis=-1):
    return jax.nn.softmax(x, axis=axis)

def _gelu(x):
    return jax.nn.gelu(x, approximate=True)

def _silu(x):
    return jax.nn.silu(x)

def _sigmoid(x):
    return jax.nn.sigmoid(x)

def _layernorm(x, axis=-1, eps=1e-05):
    m = jnp.mean(x, axis=axis, keepdims=True)
    v = jnp.var(x, axis=axis, keepdims=True)
    return (x - m) / jnp.sqrt(v + eps)

def _scatter_add(tgt, idx, src, axis=0):
    return tgt.at[idx].add(src)

def _segment_sum(src, seg, n):
    return jax.ops.segment_sum(src, seg, n)

class _Rng:

    def __init__(self, key):
        self._k = key

    def _next(self):
        self._k, sub = jax.random.split(self._k)
        return sub

    def normal(self, shape):
        return jax.random.normal(self._next(), shape, dtype=jnp.bfloat16)

    def randint(self, lo, hi, shape):
        return jax.random.randint(self._next(), shape, lo, hi, dtype=jnp.int32)

    def uniform(self, shape, lo=0.0, hi=1.0):
        return jax.random.uniform(self._next(), shape, jnp.bfloat16, lo, hi)

    def permutation(self, n):
        return jax.random.permutation(self._next(), n)
kernel_name = 'parallel_sum__memory_aug_recurrent_mem_tr__moe_arch_mod__prompt'

def setup_inputs():
    _rng = _Rng(jax.random.key(int.from_bytes(__import__("os").urandom(4), "little")))
    _w = lambda a: (lambda t: t.astype(jnp.bfloat16) if jnp.issubdtype(t.dtype, jnp.floating) else t)(jnp.asarray(a))

    def _A_setup():
        B, S, Dm = (1, 2048, 1024)
        H, Dh = (32, 128)
        M, seg = (8, 32)
        seg = min(seg, S)
        S = S // seg * seg
        return {'x': _w((lambda *s: _rng.normal(s) * 0.05)(B, S, Dm)), 'mem0': _w((lambda *s: _rng.normal(s) * 0.05)(B, M, Dm)), 'Wq': _w((lambda *s: _rng.normal(s) * 0.05)(Dm, H, Dh) * Dm ** (-0.5)), 'Wk': _w((lambda *s: _rng.normal(s) * 0.05)(Dm, H, Dh) * Dm ** (-0.5)), 'Wv': _w((lambda *s: _rng.normal(s) * 0.05)(Dm, H, Dh) * Dm ** (-0.5)), 'Wo': _w((lambda *s: _rng.normal(s) * 0.05)(H, Dh, Dm) * (H * Dh) ** (-0.5)), 'seg_len': seg}
    _A_in = _A_setup()

    def _B_setup():
        B, S, D, F, C = (1, 2048, 1024, 3584, 2)
        return {'x': _w((lambda *s: _rng.normal(s) * 0.05)(B, S, D)), 'w_r': _w((lambda *s: _rng.normal(s) * 0.05)(D)), 'w_gate': _w((lambda *s: _rng.normal(s) * 0.05)(D, F)), 'w_up': _w((lambda *s: _rng.normal(s) * 0.05)(D, F)), 'w_down': _w((lambda *s: _rng.normal(s) * 0.05)(F, D))}
    _B_in = _B_setup()
    return {'A_x': _A_in['x'], 'A_mem0': _A_in['mem0'], 'A_Wq': _A_in['Wq'], 'A_Wk': _A_in['Wk'], 'A_Wv': _A_in['Wv'], 'A_Wo': _A_in['Wo'], 'A_seg_len': _A_in['seg_len'], 'B_x': _B_in['x'], 'B_w_r': _B_in['w_r'], 'B_w_gate': _B_in['w_gate'], 'B_w_up': _B_in['w_up'], 'B_w_down': _B_in['w_down']}

def reference(A_x, A_mem0, A_Wq, A_Wk, A_Wv, A_Wo, A_seg_len, B_x, B_w_r, B_w_gate, B_w_up, B_w_down):

    def _A_ref(x, mem0, Wq, Wk, Wv, Wo, seg_len):
        B, S, Dm = x.shape
        H, Dh = (Wq.shape[1], Wq.shape[2])
        M = mem0.shape[1]
        scale = Dh ** (-0.5)
        n_seg = S // seg_len
        L = M + seg_len
        idx = jnp.arange(L)
        mask = (idx[:, None] < M) | (idx[:, None] >= idx[None, :])
        mem = mem0
        outs = []
        for s in range(n_seg):
            xs = x[:, s * seg_len:(s + 1) * seg_len, :].copy()
            h = jnp.concatenate([mem, xs], axis=1)
            q = jnp.einsum('btd,dhe->bhte', h, Wq)
            k = jnp.einsum('btd,dhe->bhte', h, Wk)
            v = jnp.einsum('btd,dhe->bhte', h, Wv)
            scores = jnp.einsum('bhqe,bhke->bhqk', q, k) * scale
            scores = jnp.where(mask[None, None], scores, -1000000000.0)
            p = _softmax(scores, axis=-1)
            o = jnp.einsum('bhqk,bhke->bhqe', p, v)
            o = jnp.einsum('bhte,hed->btd', o, Wo)
            mem = o[:, :M, :].copy()
            outs.append(o[:, M:, :])
        return jnp.concatenate(outs, axis=1)

    def _B_ref(x, w_r, w_gate, w_up, w_down):
        B, S, D = x.shape
        C = 2
        r = x @ w_r
        idx = jnp.argsort(-r, axis=-1)[:, :C]
        idx_e = jnp.repeat(idx.reshape(B, C, 1), D, axis=2)
        x_sel = jnp.take_along_axis(x, idx_e, axis=1)
        g = _silu(x_sel @ w_gate)
        u = x_sel @ w_up
        y = g * u @ w_down
        r_sel = _sigmoid(jnp.take_along_axis(r, idx, axis=1))
        y = y * r_sel.reshape(B, C, 1)
        b_off = (jnp.arange(B) * S).reshape(B, 1)
        flat_idx = (idx + b_off).reshape(B * C)
        zero = (x * 0.0).reshape(B * S, D)
        upd = _scatter_add(zero, flat_idx, y.reshape(B * C, D), axis=0)
        return x + upd.reshape(B, S, D)
    x = A_x
    xn = _layernorm(x, axis=-1)
    return x + _A_ref(xn, A_mem0, A_Wq, A_Wk, A_Wv, A_Wo, A_seg_len) + _B_ref(xn, B_w_r, B_w_gate, B_w_up, B_w_down)
```

```python
import functools

import jax
import jax.numpy as jnp
from jax import lax
import jax.experimental.pallas as pl
import jax.experimental.pallas.tpu as pltpu

F32 = jnp.float32
BF16 = jnp.bfloat16
U32 = jnp.uint32

TOP_K = 2
LN_EPS = 1e-05
MASK_VALUE = -1000000000.0


def _rbf16(x):
    return x.astype(BF16).astype(F32)


def _as_bf16(words):
    return pltpu.bitcast(words, BF16)


def _kernel(x_hbm, mem0_hbm, wq_hbm, wk_hbm, wv_hbm, wo_hbm, wr_hbm, wg_hbm, wu_hbm, wd_hbm,
            out_hbm,
            xbuf, membuf, wrbuf, hall, stage, wqkv, wo, obuf, outbuf, rbuf, wg, wu, wd,
            sem_in, sem_stage, sem_ffn, sem_out,
            *, S, D, H, Dh, M, T):
    n_seg = S // T
    L = M + T
    scale = Dh ** (-0.5)
    n_stage = stage.shape[0]
    stage_rows = stage.shape[1]
    dc = stage_rows // H
    n_chunk = D // dc

    cp_x = pltpu.make_async_copy(x_hbm, xbuf, sem_in.at[0])
    cp_mem = pltpu.make_async_copy(mem0_hbm, membuf, sem_in.at[1])
    cp_wr = pltpu.make_async_copy(wr_hbm, wrbuf, sem_in.at[2])
    cp_x.start()
    cp_mem.start()
    cp_wr.start()

    jobs = [(m, c) for m in range(3) for c in range(n_chunk)]
    w_hbm = (wq_hbm, wk_hbm, wv_hbm)

    def stage_copy(j):
        m, c = jobs[j]
        return pltpu.make_async_copy(
            w_hbm[m].at[pl.ds(c * stage_rows, stage_rows)], stage.at[j % n_stage],
            sem_stage.at[j % n_stage])

    for j in range(n_stage):
        stage_copy(j).start()

    cp_x.wait()
    cp_mem.wait()
    cp_wr.wait()
    w_r = wrbuf[...].astype(F32).reshape(1, D)

    def ln_body(s, carry):
        xs = xbuf[pl.ds(pl.multiple_of(s * T, T), T), :].astype(F32)
        mean = jnp.mean(xs, axis=-1, keepdims=True)
        cen = xs - mean
        var = jnp.mean(cen * cen, axis=-1, keepdims=True)
        den = _rbf16(jnp.sqrt(_rbf16(_rbf16(var) + LN_EPS)))
        xn = _rbf16(_rbf16(xs - _rbf16(mean)) / den)
        hall[s, M:, :] = xn
        r = _rbf16(jnp.sum(xn * w_r, axis=-1, keepdims=True))
        rbuf[pl.ds(pl.multiple_of(s * T, T), T), :] = jnp.broadcast_to(r, (T, 128))
        return carry

    lax.fori_loop(0, n_seg, ln_body, 0)
    hall[0, :M, :] = membuf[...].astype(F32)

    for j, (m, c) in enumerate(jobs):
        stage_copy(j).wait()
        s32 = stage.at[j % n_stage].bitcast(U32)
        for p in range(H // 2):
            a = s32[pl.ds(p, dc // 2, stride=H), :]
            b = s32[pl.ds(H // 2 + p, dc // 2, stride=H), :]
            lo = (a & jnp.uint32(0xFFFF)) | (b << 16)
            hi = (a >> 16) | (b & jnp.uint32(0xFFFF0000))
            rows = pl.ds(c * (dc // 2), dc // 2)
            wqkv[2 * p, rows, m * Dh:(m + 1) * Dh] = lo
            wqkv[2 * p + 1, rows, m * Dh:(m + 1) * Dh] = hi
        if j + n_stage < len(jobs):
            stage_copy(j + n_stage).start()

    wo_rows = outbuf.shape[0]
    for c in range(H * Dh // wo_rows):
        cp = pltpu.make_async_copy(wo_hbm.at[pl.ds(c * wo_rows, wo_rows)], outbuf, sem_in.at[0])
        cp.start()
        cp.wait()
        wo[pl.ds(c * (wo_rows // 2), wo_rows // 2), :] = pltpu.bitcast(outbuf[...], U32)

    cp_g = pltpu.make_async_copy(wg_hbm, wg, sem_ffn.at[0])
    cp_u = pltpu.make_async_copy(wu_hbm, wu, sem_ffn.at[1])
    cp_d = pltpu.make_async_copy(wd_hbm, wd, sem_ffn.at[2])
    cp_g.start()
    cp_u.start()
    cp_d.start()

    ri = lax.broadcasted_iota(jnp.int32, (L, L), 0)
    ci = lax.broadcasted_iota(jnp.int32, (L, L), 1)
    mask = (ri < M) | (ri >= ci)

    def out_copy(s):
        rows = pl.ds(pl.multiple_of(s * T, T), T)
        return pltpu.make_async_copy(outbuf.at[rows], out_hbm.at[rows], sem_out.at[0])

    def step(s, carry):
        qkv = {}
        prob = {}

        def do_qkv(h):
            r = jnp.dot(hall[s], _as_bf16(wqkv[h]), preferred_element_type=F32)
            qkv[h] = (r[:, :Dh], r[:, Dh:2 * Dh].astype(BF16), r[:, 2 * Dh:].astype(BF16))

        def do_scores(h):
            q, k, _ = qkv[h]
            sc = lax.dot_general(q, k, (((1,), (1,)), ((), ())), preferred_element_type=F32)
            sc = jnp.where(mask, sc * scale, MASK_VALUE)
            e = jnp.exp(sc - jnp.max(sc, axis=-1, keepdims=True))
            prob[h] = e / jnp.sum(e, axis=-1, keepdims=True)

        def do_pv(h):
            obuf[:, h * Dh:(h + 1) * Dh] = jnp.dot(prob.pop(h), qkv.pop(h)[2],
                                                   preferred_element_type=F32)

        def do_wo(k0, k1):
            return jnp.dot(obuf[:, k0:k1], _as_bf16(wo[k0 // 2:k1 // 2, :]),
                           preferred_element_type=F32)

        for h in range(H):
            do_qkv(h)
            if h >= 1:
                do_scores(h - 1)
            if h >= 2:
                do_pv(h - 2)
        o = do_wo(0, 8 * Dh)
        do_scores(H - 1)
        do_pv(H - 2)
        o = o + do_wo(8 * Dh, 16 * Dh)
        do_pv(H - 1)
        o = o + do_wo(16 * Dh, H * Dh)

        @pl.when(s + 1 < n_seg)
        def _():
            hall[s + 1, :M, :] = o[:M]

        rows = pl.ds(pl.multiple_of(s * T, T), T)
        outbuf[rows, :] = (xbuf[rows, :].astype(F32) + o[M:] + hall[s, M:, :]).astype(BF16)
        out_copy(s).start()
        return carry

    lax.fori_loop(0, n_seg, step, 0)

    tok = lax.broadcasted_iota(jnp.int32, (S, 128), 0)
    r_all = rbuf[...]
    key = jnp.where(r_all != r_all, -jnp.inf, r_all)
    m1 = jnp.max(key, axis=0, keepdims=True)
    i1v = jnp.min(jnp.where(key == m1, tok, S), axis=0, keepdims=True)
    rest = tok != i1v
    m2 = jnp.max(jnp.where(rest, key, -jnp.inf), axis=0, keepdims=True)
    i2v = jnp.min(jnp.where(rest & (key == m2), tok, S), axis=0, keepdims=True)
    idx = (jnp.max(i1v), jnp.max(i2v))

    sub = lax.broadcasted_iota(jnp.int32, (8, D), 0)
    x_sel = jnp.zeros((8, D), F32)
    r_sel = jnp.zeros((8, 128), F32)
    for n, i in enumerate(idx):
        x_sel = jnp.where(sub == n, hall[i // T, pl.ds(M + i % T, 1), :], x_sel)
        r_sel = jnp.where(sub[:, :128] == n, rbuf[pl.ds(i, 1), :], r_sel)

    cp_g.wait()
    cp_u.wait()
    cp_d.wait()
    g = jnp.dot(x_sel, wg[...], preferred_element_type=F32)
    u = jnp.dot(x_sel, wu[...], preferred_element_type=F32)
    act = g * jax.nn.sigmoid(g) * u
    y = jnp.dot(act, wd[...], preferred_element_type=F32) * jax.nn.sigmoid(r_sel[:, :1])

    pltpu.make_async_copy(outbuf, out_hbm, sem_out.at[0]).wait()
    sub16 = lax.broadcasted_iota(jnp.int32, (16, D), 0)
    for n, i in enumerate(idx):
        rows = pl.ds(pl.multiple_of(i // 16 * 16, 16), 16)
        blk = outbuf[rows, :].astype(F32)
        outbuf[rows, :] = jnp.where(sub16 == i % 16, blk + y[n:n + 1], blk).astype(BF16)
    for i in idx:
        rows = pl.ds(pl.multiple_of(i // 16 * 16, 16), 16)
        cp = pltpu.make_async_copy(outbuf.at[rows], out_hbm.at[rows], sem_out.at[0])
        cp.start()
        cp.wait()


@functools.partial(jax.jit, static_argnames=("A_seg_len",))
def pallas_parallel_sum__memory_aug_recurrent_mem_tr__moe_arch_mod__prompt_kernel(
    A_x: jax.Array,
    A_mem0: jax.Array,
    A_Wq: jax.Array,
    A_Wk: jax.Array,
    A_Wv: jax.Array,
    A_Wo: jax.Array,
    A_seg_len: int,
    B_x: jax.Array,
    B_w_r: jax.Array,
    B_w_gate: jax.Array,
    B_w_up: jax.Array,
    B_w_down: jax.Array,
):
    del B_x
    B, S, D = A_x.shape
    _, H, Dh = A_Wq.shape
    M = A_mem0.shape[1]
    T = int(A_seg_len)
    F = B_w_gate.shape[1]
    assert B == 1 and S % T == 0 and T % 16 == 0 and M % 8 == 0 and Dh == 128 and H % 2 == 0
    L = M + T
    n_seg = S // T

    any_spec = pl.BlockSpec(memory_space=pl.ANY)
    out = pl.pallas_call(
        functools.partial(_kernel, S=S, D=D, H=H, Dh=Dh, M=M, T=T),
        out_shape=jax.ShapeDtypeStruct((S, D), A_x.dtype),
        in_specs=[any_spec] * 10,
        out_specs=any_spec,
        scratch_shapes=[
            pltpu.VMEM((S, D), BF16),
            pltpu.VMEM((M, D), BF16),
            pltpu.VMEM((D,), BF16),
            pltpu.VMEM((n_seg, L, D), F32),
            pltpu.VMEM((4, 128 * H, Dh), BF16),
            pltpu.VMEM((H, D // 2, 3 * Dh), U32),
            pltpu.VMEM((H * Dh // 2, D), U32),
            pltpu.VMEM((L, H * Dh), F32),
            pltpu.VMEM((S, D), BF16),
            pltpu.VMEM((S, 128), F32),
            pltpu.VMEM((D, F), BF16),
            pltpu.VMEM((D, F), BF16),
            pltpu.VMEM((F, D), BF16),
            pltpu.SemaphoreType.DMA((3,)),
            pltpu.SemaphoreType.DMA((4,)),
            pltpu.SemaphoreType.DMA((3,)),
            pltpu.SemaphoreType.DMA((1,)),
        ],
        compiler_params=pltpu.CompilerParams(vmem_limit_bytes=110 * 1024 * 1024),
        name="rmt_mod_fused",
    )(
        A_x.reshape(S, D),
        A_mem0.reshape(M, D),
        A_Wq.reshape(D * H, Dh),
        A_Wk.reshape(D * H, Dh),
        A_Wv.reshape(D * H, Dh),
        A_Wo.reshape(H * Dh, D),
        B_w_r,
        B_w_gate,
        B_w_up,
        B_w_down,
    )
    return out.reshape(B, S, D)
```

```python
import contextlib
import functools
NSTEP = 64
SK_S = 2
SK_P = 5
LOOK = 2
G = 2
UNROLL = 1
LNU = 16
RCH = 16
NOBC = 0
SCOPES = 0
WOSPLIT = [6,12,18,24,28,32]

import jax
import jax.numpy as jnp
from jax import lax
import jax.experimental.pallas as pl
import jax.experimental.pallas.tpu as pltpu

F32 = jnp.float32
BF16 = jnp.bfloat16
U32 = jnp.uint32

LN_EPS = 1e-05
MASK_VALUE = -1000000000.0
X_EARLY = 8
PRE = 8

def scope(n):
    return jax.named_scope(n) if SCOPES else contextlib.nullcontext()

def _rbf16(x):
    return x.astype(BF16).astype(F32)


def _as_bf16(words):
    return pltpu.bitcast(words, BF16)


def _repack(w_ref, p):
    for r in range(0, w_ref.shape[1], RCH):
        a = w_ref[2 * p, r:r + RCH]
        b = w_ref[2 * p + 1, r:r + RCH]
        w_ref[2 * p, r:r + RCH] = (a & jnp.uint32(0xFFFF)) | (b << 16)
        w_ref[2 * p + 1, r:r + RCH] = (a >> 16) | (b & jnp.uint32(0xFFFF0000))


def _kernel(x_hbm, mem0_hbm, wq_hbm, wk_hbm, wv_hbm, wo_hbm, wr_hbm, wg_hbm, wu_hbm, wd_hbm,
            out_hbm,
            xbuf, membuf, wrbuf, hall, xpre, wq, wk, wv, wo, qpre, kpre, obuf, outbuf, rbuf,
            wg, wu, wd,
            sem_in, sem_qk, sem_vo, sem_ffn, sem_out,
            *, S, D, H, Dh, M, T):
    n_seg = S // T
    L = M + T
    scale = Dh ** (-0.5)
    n_grp = H // 2 // G
    seg_per_grp = n_seg // n_grp
    wo_rows = H * Dh // 2 // n_grp

    wq32, wk32, wv32, wo32 = (r.bitcast(U32) for r in (wq_hbm, wk_hbm, wv_hbm, wo_hbm))

    def qk_copies(g):
        return [pltpu.make_async_copy(src.at[:, b, g * G + t, :], dst.at[2 * (g * G + t) + b],
                                      sem_qk.at[g])
                for src, dst in ((wq32, wq), (wk32, wk)) for t in range(G) for b in range(2)]

    def vo_copies(g):
        rows = pl.ds(pl.multiple_of(g * wo_rows, wo_rows), wo_rows)
        return [pltpu.make_async_copy(wv32.at[:, b, g * G + t, :], wv.at[2 * (g * G + t) + b],
                                      sem_vo.at[g]) for t in range(G) for b in range(2)] + [
            pltpu.make_async_copy(wo32.at[rows], wo.at[rows], sem_vo.at[g])]

    def start(copies):
        for cp in copies:
            cp.start()

    def wait(copies):
        for cp in copies:
            cp.wait()

    cp_xp = pltpu.make_async_copy(x_hbm.at[:, T - PRE:, :], xbuf.at[:, T - PRE:, :], sem_in.at[0])
    cp_mem = pltpu.make_async_copy(mem0_hbm, membuf, sem_in.at[1])
    cp_wr = pltpu.make_async_copy(wr_hbm, wrbuf, sem_in.at[2])
    cp_xa = pltpu.make_async_copy(x_hbm.at[:X_EARLY, :T - PRE, :], xbuf.at[:X_EARLY, :T - PRE, :],
                                  sem_in.at[3])
    cp_xb = pltpu.make_async_copy(x_hbm.at[X_EARLY:, :T - PRE, :], xbuf.at[X_EARLY:, :T - PRE, :],
                                  sem_in.at[4])
    start([cp_xp, cp_wr, cp_mem])

    lane = lax.broadcasted_iota(jnp.int32, (8, 128), 1)

    with scope("wait0"):
        wait([cp_xp, cp_wr, cp_mem])
    start(qk_copies(0))
    w_r = wrbuf[...].astype(F32).reshape(1, D)
    hall[0, :M, :] = membuf[...].astype(F32)
    rbuf[...] = jnp.full(rbuf.shape, -jnp.inf, F32)

    def layernorm(s, r0):
        xs = xbuf[s, r0:r0 + 8, :].astype(F32)
        mean = jnp.mean(xs, axis=-1, keepdims=True)
        cen = xs - mean
        var = jnp.mean(cen * cen, axis=-1, keepdims=True)
        den = _rbf16(jnp.sqrt(_rbf16(_rbf16(var) + LN_EPS)))
        xn = _rbf16(_rbf16(xs - _rbf16(mean)) / den)
        hall[s, M + r0:M + r0 + 8, :] = xn
        return xn, _rbf16(jnp.sum(xn * w_r, axis=-1, keepdims=True))

    def layernorm_rest(s):
        for r0 in range(0, T - PRE, 8):
            _, r = layernorm(s, r0)
            rbuf[r0:r0 + 8, :] = jnp.where(lane == s, r, rbuf[r0:r0 + 8, :])

    def ln_pre(i, carry):
        r_acc = rbuf[T - PRE:, :]
        for t in range(LNU):
            s = i * LNU + t
            xn, r = layernorm(s, T - PRE)
            xpre[pl.ds(pl.multiple_of(s * PRE, PRE), PRE), :] = xn
            r_acc = jnp.where(lane == s, r, r_acc)
        rbuf[T - PRE:, :] = r_acc
        return carry

    with scope("lnpre"):
        lax.fori_loop(0, n_seg // LNU, ln_pre, 0)

    start(qk_copies(1))

    def grp_body(g, first, left):
        with scope("waitw"):
            wait(qk_copies(g))
            if not first:
                wait(vo_copies(g - 1))
        start(vo_copies(g))
        if left >= 2:
            start(qk_copies(g + 2))
        if left == 0:
            cp_xa.start()
        _repack(wq, g * G)
        for t in range(2 * G):
            h = 2 * G * g + t
            qpre[h] = jnp.dot(xpre[...], _as_bf16(wq[h]), preferred_element_type=F32)
            if t + 1 < G:
                _repack(wq, g * G + t + 1)
        for t in range(G):
            _repack(wk, g * G + t)
        for t in range(2 * G):
            h = 2 * G * g + t
            kpre[h] = jnp.dot(xpre[...], _as_bf16(wk[h]), preferred_element_type=F32)
        if not first:
            for t in range(G):
                _repack(wv, (g - 1) * G + t)

    with scope("pairs"):
        grp_body(0, True, 2)
        lax.fori_loop(1, n_grp - 2, lambda g, c: grp_body(g, False, 2), None)
        grp_body(n_grp - 2, False, 1)
        grp_body(n_grp - 1, False, 0)

    cp_g = pltpu.make_async_copy(wg_hbm.bitcast(U32), wg, sem_ffn.at[0])
    cp_u = pltpu.make_async_copy(wu_hbm.bitcast(U32), wu, sem_ffn.at[1])
    cp_d = pltpu.make_async_copy(wd_hbm.bitcast(U32), wd, sem_ffn.at[2])
    with scope("ln0"):
        wait(vo_copies(n_grp - 1))
        cp_xa.wait()
        cp_xb.start()
        for t in range(G):
            _repack(wv, (n_grp - 1) * G + t)
        layernorm_rest(0)

    ri = lax.broadcasted_iota(jnp.int32, (L, L), 0)
    ci = lax.broadcasted_iota(jnp.int32, (L, L), 1)
    mask = (ri < M) | (ri >= ci)

    def out_copy(s):
        return pltpu.make_async_copy(outbuf.at[s], out_hbm.at[s], sem_out.at[0])

    def step(s):
        qkv = {}
        prob = {}
        pre_rows = pl.ds(pl.multiple_of(s * PRE, PRE), PRE)

        def do_qkv(h):
            k = jnp.dot(hall[s, :L - PRE, :], _as_bf16(wk[h]), preferred_element_type=F32)
            q = jnp.dot(hall[s, :L - PRE, :], _as_bf16(wq[h]), preferred_element_type=F32)
            v = jnp.dot(hall[s], _as_bf16(wv[h]), preferred_element_type=F32)
            q = jnp.concatenate([q, qpre[h, pre_rows, :]], axis=0)
            k = jnp.concatenate([k, kpre[h, pre_rows, :]], axis=0)
            qkv[h] = (q, k.astype(BF16), v.astype(BF16))

        def do_scores(h):
            q, k, _ = qkv[h]
            sc = lax.dot_general(q, k, (((1,), (1,)), ((), ())), preferred_element_type=F32)
            sc = jnp.where(mask, sc * scale, MASK_VALUE)
            e = jnp.exp(sc - jnp.max(sc, axis=-1, keepdims=True))
            prob[h] = e / jnp.sum(e, axis=-1, keepdims=True)

        def do_pv(h):
            obuf[:, h * Dh:(h + 1) * Dh] = jnp.dot(prob.pop(h), qkv.pop(h)[2],
                                                   preferred_element_type=F32)

        def do_wo(h0, h1):
            return jnp.dot(obuf[:, h0 * Dh:h1 * Dh], _as_bf16(wo[h0 * Dh // 2:h1 * Dh // 2, :]),
                           preferred_element_type=F32)

        o = None
        bounds = [0] + WOSPLIT
        for i in range(H + max(SK_P, len(WOSPLIT))):
            if i < H:
                do_qkv(i)
            elif i - H < len(WOSPLIT) - 1:
                if i == H:
                    xn_s = hall[s, M:, :]
                    layernorm_rest(jnp.minimum(s + 1, n_seg - 1))
                part = do_wo(bounds[i - H], bounds[i - H + 1])
                o = part if o is None else o + part
            if 0 <= i - SK_S < H:
                do_scores(i - SK_S)
            if 0 <= i - SK_P < H:
                do_pv(i - SK_P)
        o = o + do_wo(bounds[-2], bounds[-1])

        hall[s + 1, :M, :] = o[:M]
        outbuf[s] = (xbuf[s].astype(F32) + o[M:] + xn_s).astype(BF16)

    def steps(j, carry):
        for u in range(UNROLL):
            step(j * UNROLL + u)
        for u in range(UNROLL):
            out_copy(j * UNROLL + u).start()

        @pl.when(j == (X_EARLY - 1) // UNROLL - 1)
        def _():
            cp_xb.wait()
            start([cp_g, cp_u, cp_d])
        return carry

    with scope("main"):
        lax.fori_loop(0, NSTEP // UNROLL, steps, 0)

    with scope("top2"):
        seg_id = lax.broadcasted_iota(jnp.int32, (T, 128), 1)
        tok = seg_id * T + lax.broadcasted_iota(jnp.int32, (T, 128), 0)
        r_all = rbuf[...]
        key = jnp.where(r_all != r_all, -jnp.inf, r_all)
        live = seg_id < n_seg
        idx, r_top = [], []
        for _ in range(2):
            best = jnp.max(jnp.where(live, key, -jnp.inf), keepdims=True)
            first = jnp.min(jnp.where(live & (key == best), tok, S), keepdims=True)
            r_top.append(jnp.sum(jnp.where(tok == first, r_all, 0.0), keepdims=True))
            idx.append(first[0, 0])
            live = live & (tok != first)
        seg_of = [i // T for i in idx]

    with scope("ffn"):
        sub = lax.broadcasted_iota(jnp.int32, (8, D), 0)
        x_sel = jnp.zeros((8, D), F32)
        for n, i in enumerate(idx):
            x_sel = jnp.where(sub == n, hall[i // T, pl.ds(M + i % T, 1), :], x_sel)

        wait([cp_g, cp_u, cp_d])
        g = jnp.dot(x_sel, _as_bf16(wg[...]), preferred_element_type=F32)
        u = jnp.dot(x_sel, _as_bf16(wu[...]), preferred_element_type=F32)
        act = g * jax.nn.sigmoid(g) * u
        y = jnp.dot(act, _as_bf16(wd[...]), preferred_element_type=F32)

    with scope("fin"):
        pltpu.make_async_copy(outbuf.at[:NSTEP], out_hbm.at[:NSTEP], sem_out.at[0]).wait()
        row = lax.broadcasted_iota(jnp.int32, (T, D), 0)
        for n, i in enumerate(idx):
            blk = outbuf[i // T].astype(F32)
            upd = y[n:n + 1] * jax.nn.sigmoid(r_top[n])
            outbuf[i // T] = jnp.where(row == i % T, blk + upd, blk).astype(BF16)
        out_copy(seg_of[0]).start()

        @pl.when(seg_of[1] != seg_of[0])
        def _():
            out_copy(seg_of[1]).start()
            out_copy(seg_of[1]).wait()

        out_copy(seg_of[0]).wait()


@functools.partial(jax.jit, static_argnames=("A_seg_len",))
def pallas_parallel_sum__memory_aug_recurrent_mem_tr__moe_arch_mod__prompt_kernel(
    A_x: jax.Array,
    A_mem0: jax.Array,
    A_Wq: jax.Array,
    A_Wk: jax.Array,
    A_Wv: jax.Array,
    A_Wo: jax.Array,
    A_seg_len: int,
    B_x: jax.Array,
    B_w_r: jax.Array,
    B_w_gate: jax.Array,
    B_w_up: jax.Array,
    B_w_down: jax.Array,
):
    del B_x
    B, S, D = A_x.shape
    _, H, Dh = A_Wq.shape
    M = A_mem0.shape[1]
    T = int(A_seg_len)
    F = B_w_gate.shape[1]
    L = M + T
    n_seg = S // T
    assert B == 1 and S % T == 0 and T % 16 == 0 and M % 8 == 0 and Dh == 128 and H % 2 == 0
    assert n_seg % (H // 2) == 0 and n_seg % 8 == 0 and n_seg <= 128

    any_spec = pl.BlockSpec(memory_space=pl.ANY)
    out = pl.pallas_call(
        functools.partial(_kernel, S=S, D=D, H=H, Dh=Dh, M=M, T=T),
        out_shape=jax.ShapeDtypeStruct((n_seg, T, D), A_x.dtype),
        in_specs=[any_spec] * 10,
        out_specs=any_spec,
        scratch_shapes=[
            pltpu.VMEM((n_seg, T, D), BF16),
            pltpu.VMEM((M, D), BF16),
            pltpu.VMEM((D,), BF16),
            pltpu.VMEM((n_seg + 1, L, D), F32),
            pltpu.VMEM((n_seg * PRE, D), F32),
            pltpu.VMEM((H, D // 2, Dh), U32),
            pltpu.VMEM((H, D // 2, Dh), U32),
            pltpu.VMEM((H, D // 2, Dh), U32),
            pltpu.VMEM((H * Dh // 2, D), U32),
            pltpu.VMEM((H, n_seg * PRE, Dh), F32),
            pltpu.VMEM((H, n_seg * PRE, Dh), F32),
            pltpu.VMEM((L, H * Dh), F32),
            pltpu.VMEM((n_seg, T, D), BF16),
            pltpu.VMEM((T, 128), F32),
            pltpu.VMEM((D // 2, F), U32),
            pltpu.VMEM((D // 2, F), U32),
            pltpu.VMEM((F // 2, D), U32),
            pltpu.SemaphoreType.DMA((5,)),
            pltpu.SemaphoreType.DMA((H // 2 // G,)),
            pltpu.SemaphoreType.DMA((H // 2 // G,)),
            pltpu.SemaphoreType.DMA((3,)),
            pltpu.SemaphoreType.DMA((1,)),
        ],
        compiler_params=pltpu.CompilerParams(vmem_limit_bytes=120 * 1024 * 1024,
                                             disable_bounds_checks=bool(NOBC)),
        name="rmt_mod_fused",
    )(
        A_x.reshape(n_seg, T, D),
        A_mem0.reshape(M, D),
        A_Wq.reshape(D // 2, 2, H, Dh),
        A_Wk.reshape(D // 2, 2, H, Dh),
        A_Wv.reshape(D // 2, 2, H, Dh),
        A_Wo.reshape(H * Dh, D),
        B_w_r,
        B_w_gate,
        B_w_up,
        B_w_down,
    )
    return out.reshape(B, S, D)
```

```python
import contextlib
import functools


SCOPES = 0
UNROLL = 2
SK_S = 2
SK_P = 5
HA = 24
NX = 2
PLAN_X = [(1, 0, 0), (1, 0, 0)]
GROUPS = [(1, 0), (1, 0), (2, 0), (4, 2), (4, 5), (2, 6), (2, 3)]
PLAN = [(2, 0, 0), (2, 0, 0), (2, 2, 0), (4, 5, 0), (4, 6, 0), (0, 3, 4), (0, 0, 12)]
FFN_AT = [32,33,34,35,38,39]

import jax
import jax.numpy as jnp
from jax import lax
import jax.experimental.pallas as pl
import jax.experimental.pallas.tpu as pltpu

F32 = jnp.float32
BF16 = jnp.bfloat16
U32 = jnp.uint32

TOP_K = 2
LN_EPS = 1e-05
MASK_VALUE = -1000000000.0
PRE = 8


def scope(n):
    return jax.named_scope(n) if SCOPES else contextlib.nullcontext()


def _rbf16(x):
    return x.astype(BF16).astype(F32)


def _dot(lhs, words):
    return jnp.dot(lhs, pltpu.bitcast(words, BF16), preferred_element_type=F32)


def _split_pair(w_ref, p):
    for r in range(0, w_ref.shape[1], 16):
        a = w_ref[2 * p, r:r + 16]
        b = w_ref[2 * p + 1, r:r + 16]
        w_ref[2 * p, r:r + 16] = (a & jnp.uint32(0xFFFF)) | (b << 16)
        w_ref[2 * p + 1, r:r + 16] = (a >> 16) | (b & jnp.uint32(0xFFFF0000))


def _start(copies):
    for cp in copies:
        cp.start()


def _wait(copies):
    for cp in copies:
        cp.wait()


def _kernel(x_hbm, mem0_hbm, wq_hbm, wk_hbm, wv_hbm, wo_hbm, wr_hbm, wg_hbm, wu_hbm, wd_hbm,
            out_hbm,
            xbuf, membuf, wrbuf, hall, wq, wk, wv, wo, qpre, kpre, obuf, outbuf, rbuf,
            wg, wu, wd, xsel, yacc, gu,
            sem_x, sem_in, sem_qk, sem_v, sem_o, sem_ffn, sem_out):
    n_seg, T, D = xbuf.shape
    M = membuf.shape[0]
    H, _, Dh = wq.shape
    L = M + T
    scale = Dh ** (-0.5)
    n_pair = H // 2
    seg_per_pair = n_seg // n_pair

    wq32, wk32, wv32, wo32 = (r.bitcast(U32) for r in (wq_hbm, wk_hbm, wv_hbm, wo_hbm))

    def qk_copies(p):
        return [pltpu.make_async_copy(src.at[:, b, p, :], dst.at[2 * p + b], sem_qk.at[p])
                for src, dst in ((wq32, wq), (wk32, wk)) for b in range(2)]

    def vx_copies(p):
        segs = pl.ds(p * seg_per_pair, seg_per_pair)
        return [pltpu.make_async_copy(wv32.at[:, b, p, :], wv.at[2 * p + b], sem_v.at[p])
                for b in range(2)] + [
                    pltpu.make_async_copy(x_hbm.at[segs, :T - PRE, :], xbuf.at[segs, :T - PRE, :],
                                          sem_v.at[p])]

    def o_copies(p):
        rows = pl.ds(p * Dh, Dh)
        return [pltpu.make_async_copy(wo32.at[rows], wo.at[rows], sem_o.at[p])]

    issued = [0, 0, 0]

    def issue(plan):
        for kind, copies in enumerate((qk_copies, vx_copies, o_copies)):
            for p in range(issued[kind], issued[kind] + plan[kind]):
                _start(copies(p))
            issued[kind] += plan[kind]

    x_seg = n_seg // NX
    cp_xp = [pltpu.make_async_copy(x_hbm.at[c * x_seg:(c + 1) * x_seg, T - PRE:, :],
                                   xbuf.at[c * x_seg:(c + 1) * x_seg, T - PRE:, :], sem_x.at[c])
             for c in range(NX)]
    cp_small = [pltpu.make_async_copy(mem0_hbm, membuf, sem_in.at[0]),
                pltpu.make_async_copy(wr_hbm, wrbuf, sem_in.at[1])]
    cp_ffn = [pltpu.make_async_copy(src.bitcast(U32), dst, sem_ffn.at[n])
              for n, (src, dst) in enumerate(((wg_hbm, wg), (wu_hbm, wu), (wd_hbm, wd)))]

    def layernorm(s, r0):
        xs = xbuf[s, r0:r0 + 8, :].astype(F32)
        mean = jnp.mean(xs, axis=-1, keepdims=True)
        cen = xs - mean
        var = jnp.mean(cen * cen, axis=-1, keepdims=True)
        den = _rbf16(jnp.sqrt(_rbf16(_rbf16(var) + LN_EPS)))
        xn = _rbf16(_rbf16(xs - _rbf16(mean)) / den)
        hall[s, M + r0:M + r0 + 8, :] = xn
        return xn

    def finish_segment(s):
        lane = lax.broadcasted_iota(jnp.int32, (8, 128), 1)
        w_r = wrbuf[...].astype(F32).reshape(1, D)
        for r0 in range(0, T, 8):
            xn = layernorm(s, r0) if r0 < T - PRE else hall[s, M + r0:M + r0 + 8, :]
            r = _rbf16(jnp.sum(xn * w_r, axis=-1, keepdims=True))
            rbuf[r0:r0 + 8, :] = jnp.where(lane == s, r, rbuf[r0:r0 + 8, :])

    cp_xp[0].start()
    _start(cp_small)
    if NX > 1:
        cp_xp[1].start()
    for c in range(NX):
        with scope("waitx"):
            cp_xp[c].wait()
        if c + 2 < NX:
            cp_xp[c + 2].start()
        issue(PLAN_X[c])
        with scope("lnpre"):
            for s in range(c * x_seg, (c + 1) * x_seg):
                layernorm(s, T - PRE)

    _wait(cp_small)
    hall[0, :M, :] = membuf[...].astype(F32)
    rbuf[...] = jnp.full(rbuf.shape, -jnp.inf, F32)
    p0 = v0 = 0
    with scope("pairs"):
        for (n_qk, n_v), plan in zip(GROUPS, PLAN):
            with scope("waitw"):
                for p in range(p0, p0 + n_qk):
                    _wait(qk_copies(p))
                for p in range(v0, v0 + n_v):
                    _wait(vx_copies(p))
            issue(plan)
            with scope("grp"):
                for w_ref, pre in ((wq, qpre), (wk, kpre)):
                    for p in range(p0, p0 + n_qk):
                        _split_pair(w_ref, p)
                    for h in range(2 * p0, 2 * (p0 + n_qk)):
                        pre[h] = _dot(hall[:n_seg, L - PRE:, :].reshape(n_seg * PRE, D), w_ref[h])
                for p in range(v0, v0 + n_v):
                    _split_pair(wv, p)
                    for s in range(p * seg_per_pair, (p + 1) * seg_per_pair):
                        finish_segment(s)
            p0 += n_qk
            v0 += n_v
    assert p0 == v0 == n_pair and issued == [n_pair] * 3

    def route():
        seg_id = lax.broadcasted_iota(jnp.int32, (T, 128), 1)
        tok = seg_id * T + lax.broadcasted_iota(jnp.int32, (T, 128), 0)
        r_all = rbuf[...]
        key = jnp.where(r_all != r_all, -jnp.inf, r_all)
        live = seg_id < n_seg
        sub = lax.broadcasted_iota(jnp.int32, (8, D), 0)
        x_sel = jnp.zeros((8, D), F32)
        idx, gate = [], []
        for n in range(TOP_K):
            best = jnp.max(jnp.where(live, key, -jnp.inf), keepdims=True)
            first = jnp.min(jnp.where(live & (key == best), tok, n_seg * T), keepdims=True)
            live = live & (tok != first)
            i = first[0, 0]
            x_sel = jnp.where(sub == n, hall[i // T, pl.ds(M + i % T, 1), :], x_sel)
            idx.append(i)
            gate.append(jax.nn.sigmoid(best))
        xsel[...] = x_sel
        yacc[...] = jnp.zeros(yacc.shape, F32)
        gu[...] = jnp.zeros(gu.shape, F32)
        return idx, gate

    n_ffn = wg.shape[1] // 128

    def step(s, ffn_slice=None, before_wo=None):
        ri = lax.broadcasted_iota(jnp.int32, (L, L), 0)
        ci = lax.broadcasted_iota(jnp.int32, (L, L), 1)
        mask = (ri < M) | (ri >= ci)
        pre_rows = pl.ds(pl.multiple_of(s * PRE, PRE), PRE)
        qkv, prob, act = {}, {}, []

        def project(h):
            k = _dot(hall[s, :L - PRE, :], wk[h])
            q = _dot(hall[s, :L - PRE, :], wq[h])
            v = _dot(hall[s], wv[h])
            q = jnp.concatenate([q, qpre[h, pre_rows, :]], axis=0)
            k = jnp.concatenate([k, kpre[h, pre_rows, :]], axis=0)
            qkv[h] = (q, k.astype(BF16), v.astype(BF16))

        def scores(h):
            q, k, _ = qkv[h]
            sc = lax.dot_general(q, k, (((1,), (1,)), ((), ())), preferred_element_type=F32)
            sc = jnp.where(mask, sc * scale, MASK_VALUE)
            e = jnp.exp(sc - jnp.max(sc, axis=-1, keepdims=True))
            prob[h] = e / jnp.sum(e, axis=-1, keepdims=True)

        def mix(h):
            obuf[:, h * Dh:(h + 1) * Dh] = jnp.dot(prob.pop(h), qkv.pop(h)[2],
                                                   preferred_element_type=F32)

        def out_proj(h0, h1, c0, c1):
            return _dot(obuf[:, h0 * Dh:h1 * Dh], wo[h0 * Dh // 2:h1 * Dh // 2, c0:c1])

        def ffn_piece(piece):
            t, slot = ffn_slice
            lag = gu.shape[0]
            half = D // 2
            if piece == 0:
                g = gu[slot, 0] + gu[slot, 1]
                act.append(g * jax.nn.sigmoid(g) * (gu[slot, 2] + gu[slot, 3]))
            if piece < 4:
                w_ref, k0 = (wg, wu)[piece // 2], piece % 2 * half
                cols = pl.ds(pl.multiple_of(jnp.minimum(t, n_ffn - 1) * 128, 128), 128)
                gu[slot, piece] = _dot(xsel[:, k0:k0 + half], w_ref[k0 // 2:(k0 + half) // 2, cols])
            else:
                c0 = piece % 2 * half
                rows = pl.ds(pl.multiple_of(jnp.maximum(t - lag, 0) * 64, 64), 64)
                part = _dot(act[0], wd[rows, c0:c0 + half])
                yacc[:, c0:c0 + half] += jnp.where(t >= lag, part, 0.0)

        parts = []
        for i in range(H + D // 128):
            if i < H:
                project(i)
            else:
                if i == H and before_wo is not None:
                    before_wo()
                parts.append(out_proj(0, HA, (i - H) * 128, (i - H + 1) * 128))
            if ffn_slice is not None and i in FFN_AT:
                ffn_piece(FFN_AT.index(i))
            if 0 <= i - SK_S < H:
                scores(i - SK_S)
            if 0 <= i - SK_P < H:
                mix(i - SK_P)
        o = jnp.concatenate(parts, axis=1) + out_proj(HA, H, 0, D)

        hall[s + 1, :M, :] = o[:M]
        outbuf[s] = (xbuf[s].astype(F32) + o[M:] + hall[s, M:, :]).astype(BF16)

    def wo_arrived():
        for p in range(n_pair):
            _wait(o_copies(p))
        _start(cp_ffn)

    with scope("first"):
        step(0, before_wo=wo_arrived)
        idx, gate = route()
        step(1)

    s_last = n_seg - 2
    s_ffn = s_last - n_ffn - UNROLL
    assert s_ffn >= 2 and (s_ffn - 2) % UNROLL == 0 and n_ffn % UNROLL == 0

    def plain_steps(j, carry):
        for u in range(UNROLL):
            step(2 + UNROLL * j + u)
        return carry

    def ffn_steps(j, carry):
        for u in range(UNROLL):
            step(s_ffn + UNROLL * j + u, ffn_slice=(UNROLL * j + u, u))
        return carry

    with scope("loop_a"):
        lax.fori_loop(0, (s_ffn - 2) // UNROLL, plain_steps, 0)
    _wait(cp_ffn)
    with scope("loop_b"):
        lax.fori_loop(0, (s_last - s_ffn) // UNROLL, ffn_steps, 0)

    def write_out(s0, s1, sem):
        row = lax.broadcasted_iota(jnp.int32, (T, D), 0)
        for n, i in enumerate(idx):
            @pl.when((i >= s0 * T) & (i < s1 * T))
            def _():
                blk = outbuf[i // T].astype(F32)
                upd = yacc[n:n + 1, :] * gate[n]
                outbuf[i // T] = jnp.where(row == i % T, blk + upd, blk).astype(BF16)
        cp = pltpu.make_async_copy(outbuf.at[s0:s1], out_hbm.at[s0:s1], sem)
        cp.start()
        return cp

    with scope("last"):
        cp_head = write_out(0, s_last, sem_out.at[0])
        for s in range(s_last, n_seg):
            step(s)
    with scope("fin"):
        _wait([cp_head, write_out(s_last, n_seg, sem_out.at[1])])


@functools.partial(jax.jit, static_argnames=("A_seg_len",))
def pallas_parallel_sum__memory_aug_recurrent_mem_tr__moe_arch_mod__prompt_kernel(
    A_x: jax.Array,
    A_mem0: jax.Array,
    A_Wq: jax.Array,
    A_Wk: jax.Array,
    A_Wv: jax.Array,
    A_Wo: jax.Array,
    A_seg_len: int,
    B_x: jax.Array,
    B_w_r: jax.Array,
    B_w_gate: jax.Array,
    B_w_up: jax.Array,
    B_w_down: jax.Array,
):
    del B_x
    B, S, D = A_x.shape
    _, H, Dh = A_Wq.shape
    M = A_mem0.shape[1]
    T = int(A_seg_len)
    F = B_w_gate.shape[1]
    L = M + T
    n_seg = S // T
    assert B == 1 and S % T == 0 and T % 16 == 0 and M % 8 == 0 and Dh == 128 and H % 2 == 0
    assert n_seg % (H // 2) == 0 and n_seg <= 128

    any_spec = pl.BlockSpec(memory_space=pl.ANY)
    out = pl.pallas_call(
        _kernel,
        out_shape=jax.ShapeDtypeStruct((n_seg, T, D), A_x.dtype),
        in_specs=[any_spec] * 10,
        out_specs=any_spec,
        scratch_shapes=[
            pltpu.VMEM((n_seg, T, D), BF16),
            pltpu.VMEM((M, D), BF16),
            pltpu.VMEM((D,), BF16),
            pltpu.VMEM((n_seg + 1, L, D), F32),
            pltpu.VMEM((H, D // 2, Dh), U32),
            pltpu.VMEM((H, D // 2, Dh), U32),
            pltpu.VMEM((H, D // 2, Dh), U32),
            pltpu.VMEM((H * Dh // 2, D), U32),
            pltpu.VMEM((H, n_seg * PRE, Dh), F32),
            pltpu.VMEM((H, n_seg * PRE, Dh), F32),
            pltpu.VMEM((L, H * Dh), F32),
            pltpu.VMEM((n_seg, T, D), BF16),
            pltpu.VMEM((T, 128), F32),
            pltpu.VMEM((D // 2, F), U32),
            pltpu.VMEM((D // 2, F), U32),
            pltpu.VMEM((F // 2, D), U32),
            pltpu.VMEM((8, D), F32),
            pltpu.VMEM((8, D), F32),
            pltpu.VMEM((UNROLL, 4, 8, 128), F32),
            pltpu.SemaphoreType.DMA((NX,)),
            pltpu.SemaphoreType.DMA((2,)),
            pltpu.SemaphoreType.DMA((H // 2,)),
            pltpu.SemaphoreType.DMA((H // 2,)),
            pltpu.SemaphoreType.DMA((H // 2,)),
            pltpu.SemaphoreType.DMA((3,)),
            pltpu.SemaphoreType.DMA((2,)),
        ],
        compiler_params=pltpu.CompilerParams(vmem_limit_bytes=120 * 1024 * 1024),
        name="rmt_mod_fused",
    )(
        A_x.reshape(n_seg, T, D),
        A_mem0.reshape(M, D),
        A_Wq.reshape(D // 2, 2, H, Dh),
        A_Wk.reshape(D // 2, 2, H, Dh),
        A_Wv.reshape(D // 2, 2, H, Dh),
        A_Wo.reshape(H * Dh, D),
        B_w_r,
        B_w_gate,
        B_w_up,
        B_w_down,
    )
    return out.reshape(B, S, D)
```

```python
import contextlib
import functools


SCOPES = 0
UNROLL = 2
SK_S = 2
SK_P = 5
CHAIN = 1
HA = 24
NX = 2
PLAN_X = [(1, 0, 0), (1, 0, 0)]
GROUPS = [(1,), (1,), (2,), (2,), (4,), (3,), (3,)]
PLAN = [(2, 0, 0), (2, 0, 0), (4, 0, 0), (3, 0, 0), (2, 8, 0), (1, 8, 2), (0, 0, 14)]
FFN_AT = [32,33,34,35,38,39]

import jax
import jax.numpy as jnp
from jax import lax
import jax.experimental.pallas as pl
import jax.experimental.pallas.tpu as pltpu

F32 = jnp.float32
BF16 = jnp.bfloat16
U32 = jnp.uint32

TOP_K = 2
LN_EPS = 1e-05
MASK_VALUE = -1000000000.0
PRE = 8


def scope(n):
    return jax.named_scope(n) if SCOPES else contextlib.nullcontext()


def _rbf16(x):
    return x.astype(BF16).astype(F32)


def _dot(lhs, words):
    return jnp.dot(lhs, pltpu.bitcast(words, BF16), preferred_element_type=F32)


def _split_pair(w_ref, p):
    for r in range(0, w_ref.shape[1], 16):
        a = w_ref[2 * p, r:r + 16]
        b = w_ref[2 * p + 1, r:r + 16]
        w_ref[2 * p, r:r + 16] = (a & jnp.uint32(0xFFFF)) | (b << 16)
        w_ref[2 * p + 1, r:r + 16] = (a >> 16) | (b & jnp.uint32(0xFFFF0000))


def _start(copies):
    for cp in copies:
        cp.start()


def _wait(copies):
    for cp in copies:
        cp.wait()


def _kernel(x_hbm, mem0_hbm, wq_hbm, wk_hbm, wv_hbm, wo_hbm, wr_hbm, wg_hbm, wu_hbm, wd_hbm,
            out_hbm,
            xbuf, membuf, wrbuf, hall, wq, wk, wv, wo, qpre, kpre, obuf, outbuf, rbuf,
            wg, wu, wd, xsel, yacc, gu,
            sem_x, sem_in, sem_qk, sem_v, sem_o, sem_ffn, sem_out):
    n_seg, T, D = xbuf.shape
    M = membuf.shape[0]
    H, _, Dh = wq.shape
    L = M + T
    scale = Dh ** (-0.5)
    n_pair = H // 2

    wq32, wk32, wv32, wo32 = (r.bitcast(U32) for r in (wq_hbm, wk_hbm, wv_hbm, wo_hbm))

    def qk_copies(p):
        return [pltpu.make_async_copy(src.at[:, b, p, :], dst.at[2 * p + b], sem_qk.at[p])
                for src, dst in ((wq32, wq), (wk32, wk)) for b in range(2)]

    def v_copies(p):
        return [pltpu.make_async_copy(wv32.at[:, b, p, :], wv.at[2 * p + b], sem_v.at[p])
                for b in range(2)]

    def o_copies(p):
        rows = pl.ds(p * Dh, Dh)
        return [pltpu.make_async_copy(wo32.at[rows], wo.at[rows], sem_o.at[p])]

    issued = [0, 0, 0]

    def issue(plan):
        for kind, copies in enumerate((qk_copies, v_copies, o_copies)):
            for p in range(issued[kind], issued[kind] + plan[kind]):
                _start(copies(p))
            issued[kind] += plan[kind]

    x_seg = n_seg // NX
    cp_xp = [pltpu.make_async_copy(x_hbm.at[c * x_seg:(c + 1) * x_seg, T - PRE:, :],
                                   xbuf.at[c * x_seg:(c + 1) * x_seg, T - PRE:, :], sem_x.at[c])
             for c in range(NX)]
    cp_small = [pltpu.make_async_copy(mem0_hbm, membuf, sem_in.at[0]),
                pltpu.make_async_copy(wr_hbm, wrbuf, sem_in.at[1])]

    def x_rest(s0, s1, sem):
        return pltpu.make_async_copy(x_hbm.at[s0:s1, :T - PRE, :], xbuf.at[s0:s1, :T - PRE, :], sem)

    half_seg = n_seg // 2
    cp_xa = [x_rest(0, 3, sem_in.at[2]), x_rest(half_seg + 1, half_seg + 2, sem_in.at[3])]
    cp_xb = [x_rest(3, half_seg + 1, sem_in.at[4]), x_rest(half_seg + 2, n_seg, sem_in.at[5])]
    cp_ffn = [pltpu.make_async_copy(src.bitcast(U32), dst, sem_ffn.at[n])
              for n, (src, dst) in enumerate(((wg_hbm, wg), (wu_hbm, wu), (wd_hbm, wd)))]

    def layernorm(s, r0, after=None):
        xs = xbuf[s, r0:r0 + 8, :].astype(F32)
        mean = jnp.mean(xs, axis=-1, keepdims=True)
        if after is not None and CHAIN:
            mean = jnp.where(after > 0, mean, mean + 0.0)
        cen = xs - mean
        var = jnp.mean(cen * cen, axis=-1, keepdims=True)
        den = _rbf16(jnp.sqrt(_rbf16(_rbf16(var) + LN_EPS)))
        xn = _rbf16(_rbf16(xs - _rbf16(mean)) / den)
        hall[s, M + r0:M + r0 + 8, :] = xn
        return xn

    def finish_segments(segs):
        lane = lax.broadcasted_iota(jnp.int32, (8, 128), 1)
        w_r = wrbuf[...].astype(F32).reshape(1, D)
        r = None
        for s in segs:
            for r0 in range(0, T, 8):
                xn = layernorm(s, r0, r) if r0 < T - PRE else hall[s, M + r0:M + r0 + 8, :]
                r = _rbf16(jnp.sum(xn * w_r, axis=-1, keepdims=True))
                rbuf[r0:r0 + 8, :] = jnp.where(lane == s, r, rbuf[r0:r0 + 8, :])

    cp_xp[0].start()
    _start(cp_small)
    if NX > 1:
        cp_xp[1].start()
    for c in range(NX):
        with scope("waitx"):
            cp_xp[c].wait()
        if c + 2 < NX:
            cp_xp[c + 2].start()
        issue(PLAN_X[c])
        with scope("lnpre"):
            for s in range(c * x_seg, (c + 1) * x_seg):
                layernorm(s, T - PRE)

    _wait(cp_small)
    hall[0, :M, :] = membuf[...].astype(F32)
    rbuf[...] = jnp.full(rbuf.shape, -jnp.inf, F32)
    p0 = 0
    with scope("pairs"):
        for (n_qk,), plan in zip(GROUPS, PLAN):
            with scope("waitw"):
                for p in range(p0, p0 + n_qk):
                    _wait(qk_copies(p))
            issue(plan)
            if p0 + n_qk + GROUPS[-1][0] == n_pair:
                _start(cp_xa)
            with scope("grp"):
                for w_ref, pre in ((wq, qpre), (wk, kpre)):
                    for p in range(p0, p0 + n_qk):
                        _split_pair(w_ref, p)
                    for h in range(2 * p0, 2 * (p0 + n_qk)):
                        pre[h] = _dot(hall[:, L - PRE:, :].reshape(n_seg * PRE, D), w_ref[h])
            p0 += n_qk
    assert p0 == n_pair and issued == [n_pair] * 3
    with scope("ln0"):
        _wait(cp_xa)
        for p in range(n_pair):
            _wait(v_copies(p))
        finish_segments([0])

    def route():
        seg_id = lax.broadcasted_iota(jnp.int32, (T, 128), 1)
        tok = seg_id * T + lax.broadcasted_iota(jnp.int32, (T, 128), 0)
        r_all = rbuf[...]
        key = jnp.where(r_all != r_all, -jnp.inf, r_all)
        live = seg_id < n_seg
        sub = lax.broadcasted_iota(jnp.int32, (8, D), 0)
        x_sel = jnp.zeros((8, D), F32)
        idx, gate = [], []
        for n in range(TOP_K):
            best = jnp.max(jnp.where(live, key, -jnp.inf), keepdims=True)
            first = jnp.min(jnp.where(live & (key == best), tok, n_seg * T), keepdims=True)
            live = live & (tok != first)
            i = first[0, 0]
            x_sel = jnp.where(sub == n, hall[i // T, pl.ds(M + i % T, 1), :], x_sel)
            idx.append(i)
            gate.append(jax.nn.sigmoid(best))
        xsel[...] = x_sel
        yacc[...] = jnp.zeros(yacc.shape, F32)
        return idx, gate

    n_ffn = wg.shape[1] // 128

    def step(s, ffn_slice=None, first=False, last=False):
        q0 = M if last else 0
        ri = q0 + lax.broadcasted_iota(jnp.int32, (L - q0, L), 0)
        ci = lax.broadcasted_iota(jnp.int32, (L - q0, L), 1)
        mask = (ri < M) | (ri >= ci)
        pre_rows = pl.ds(pl.multiple_of(s * PRE, PRE), PRE)
        qkv, prob, act = {}, {}, []

        def project(h):
            if first and h % 2 == 0:
                _split_pair(wv, h // 2)
            k = _dot(hall[s, :L - PRE, :], wk[h])
            q = _dot(hall[s, :L - PRE, :], wq[h])
            v = _dot(hall[s], wv[h])
            q = jnp.concatenate([q, qpre[h, pre_rows, :]], axis=0)
            k = jnp.concatenate([k, kpre[h, pre_rows, :]], axis=0)
            qkv[h] = (q[q0:], k.astype(BF16), v.astype(BF16))

        def scores(h):
            q, k, _ = qkv[h]
            sc = lax.dot_general(q, k, (((1,), (1,)), ((), ())), preferred_element_type=F32)
            sc = jnp.where(mask, sc * scale, MASK_VALUE)
            e = jnp.exp(sc - jnp.max(sc, axis=-1, keepdims=True))
            prob[h] = e / jnp.sum(e, axis=-1, keepdims=True)

        def mix(h):
            obuf[q0:, h * Dh:(h + 1) * Dh] = jnp.dot(prob.pop(h), qkv.pop(h)[2],
                                                     preferred_element_type=F32)

        def out_proj(h0, h1, c0, c1):
            return _dot(obuf[q0:, h0 * Dh:h1 * Dh], wo[h0 * Dh // 2:h1 * Dh // 2, c0:c1])

        def ffn_piece(piece):
            t, slot, down = ffn_slice
            half = D // 2
            if piece == 0 and down:
                g = gu[slot, 0] + gu[slot, 1]
                act.append(g * jax.nn.sigmoid(g) * (gu[slot, 2] + gu[slot, 3]))
            if piece < 4:
                w_ref, k0 = (wg, wu)[piece // 2], piece % 2 * half
                cols = pl.ds(pl.multiple_of(jnp.minimum(t, n_ffn - 1) * 128, 128), 128)
                gu[slot, piece] = _dot(xsel[:, k0:k0 + half], w_ref[k0 // 2:(k0 + half) // 2, cols])
            elif down:
                c0 = piece % 2 * half
                rows = pl.ds(pl.multiple_of((t - UNROLL) * 64, 64), 64)
                yacc[:, c0:c0 + half] += _dot(act[0], wd[rows, c0:c0 + half])

        parts = []
        for i in range(H + D // 128):
            if i < H:
                project(i)
            else:
                if i == H and first:
                    for p in range(n_pair):
                        _wait(o_copies(p))
                    _start(cp_xb)
                parts.append(out_proj(0, HA, (i - H) * 128, (i - H + 1) * 128))
            if ffn_slice is not None and i in FFN_AT:
                ffn_piece(FFN_AT.index(i))
            if 0 <= i - SK_S < H:
                scores(i - SK_S)
            if 0 <= i - SK_P < H:
                mix(i - SK_P)
        o = jnp.concatenate(parts, axis=1) + out_proj(HA, H, 0, D)

        if not last:
            hall[s + 1, :M, :] = o[:M]
        outbuf[s] = (xbuf[s].astype(F32) + o[M - q0:] + hall[s, M:, :]).astype(BF16)

    with scope("first"):
        step(0, first=True)
        finish_segments([1])
        step(1)
        finish_segments([2, half_seg + 1])
        _wait(cp_xb)
        _start(cp_ffn)

    s_last = n_seg - 2
    s_ffn = s_last - n_ffn - UNROLL
    assert s_ffn == half_seg and (s_ffn - 2) % UNROLL == 0 and n_ffn % UNROLL == 0

    def norm_steps(j, carry):
        for u in range(UNROLL):
            s = 2 + UNROLL * j + u
            step(s)
            finish_segments([s + 1, s + half_seg])
        return carry

    def ffn_steps(j, carry):
        for u in range(UNROLL):
            step(s_ffn + UNROLL * j + u, ffn_slice=(UNROLL * j + u, u, True))
        return carry

    with scope("loop_a"):
        lax.fori_loop(0, (s_ffn - 2) // UNROLL, norm_steps, 0)
    with scope("route"):
        _wait(cp_ffn)
        idx, gate = route()
        for u in range(UNROLL):
            step(s_ffn + u, ffn_slice=(u, u, False))
    with scope("loop_b"):
        lax.fori_loop(1, (s_last - s_ffn) // UNROLL, ffn_steps, 0)

    def write_out(s0, s1, sem):
        row = lax.broadcasted_iota(jnp.int32, (T, D), 0)
        for n, i in enumerate(idx):
            @pl.when((i >= s0 * T) & (i < s1 * T))
            def _():
                blk = outbuf[i // T].astype(F32)
                upd = yacc[n:n + 1, :] * gate[n]
                outbuf[i // T] = jnp.where(row == i % T, blk + upd, blk).astype(BF16)
        cp = pltpu.make_async_copy(outbuf.at[s0:s1], out_hbm.at[s0:s1], sem)
        cp.start()
        return cp

    with scope("last"):
        cp_head = write_out(0, s_last, sem_out.at[0])
        for s in range(s_last, n_seg):
            step(s, last=s == n_seg - 1)
    with scope("fin"):
        _wait([cp_head, write_out(s_last, n_seg, sem_out.at[1])])


@functools.partial(jax.jit, static_argnames=("A_seg_len",))
def pallas_parallel_sum__memory_aug_recurrent_mem_tr__moe_arch_mod__prompt_kernel(
    A_x: jax.Array,
    A_mem0: jax.Array,
    A_Wq: jax.Array,
    A_Wk: jax.Array,
    A_Wv: jax.Array,
    A_Wo: jax.Array,
    A_seg_len: int,
    B_x: jax.Array,
    B_w_r: jax.Array,
    B_w_gate: jax.Array,
    B_w_up: jax.Array,
    B_w_down: jax.Array,
):
    del B_x
    B, S, D = A_x.shape
    _, H, Dh = A_Wq.shape
    M = A_mem0.shape[1]
    T = int(A_seg_len)
    F = B_w_gate.shape[1]
    L = M + T
    n_seg = S // T
    assert B == 1 and S % T == 0 and T % 16 == 0 and M % 8 == 0 and Dh == 128 and H % 2 == 0
    assert n_seg % (H // 2) == 0 and n_seg <= 128

    any_spec = pl.BlockSpec(memory_space=pl.ANY)
    out = pl.pallas_call(
        _kernel,
        out_shape=jax.ShapeDtypeStruct((n_seg, T, D), A_x.dtype),
        in_specs=[any_spec] * 10,
        out_specs=any_spec,
        scratch_shapes=[
            pltpu.VMEM((n_seg, T, D), BF16),
            pltpu.VMEM((M, D), BF16),
            pltpu.VMEM((D,), BF16),
            pltpu.VMEM((n_seg, L, D), F32),
            pltpu.VMEM((H, D // 2, Dh), U32),
            pltpu.VMEM((H, D // 2, Dh), U32),
            pltpu.VMEM((H, D // 2, Dh), U32),
            pltpu.VMEM((H * Dh // 2, D), U32),
            pltpu.VMEM((H, n_seg * PRE, Dh), F32),
            pltpu.VMEM((H, n_seg * PRE, Dh), F32),
            pltpu.VMEM((L, H * Dh), F32),
            pltpu.VMEM((n_seg, T, D), BF16),
            pltpu.VMEM((T, 128), F32),
            pltpu.VMEM((D // 2, F), U32),
            pltpu.VMEM((D // 2, F), U32),
            pltpu.VMEM((F // 2, D), U32),
            pltpu.VMEM((8, D), F32),
            pltpu.VMEM((8, D), F32),
            pltpu.VMEM((UNROLL, 4, 8, 128), F32),
            pltpu.SemaphoreType.DMA((NX,)),
            pltpu.SemaphoreType.DMA((6,)),
            pltpu.SemaphoreType.DMA((H // 2,)),
            pltpu.SemaphoreType.DMA((H // 2,)),
            pltpu.SemaphoreType.DMA((H // 2,)),
            pltpu.SemaphoreType.DMA((3,)),
            pltpu.SemaphoreType.DMA((2,)),
        ],
        compiler_params=pltpu.CompilerParams(vmem_limit_bytes=120 * 1024 * 1024),
        name="rmt_mod_fused",
    )(
        A_x.reshape(n_seg, T, D),
        A_mem0.reshape(M, D),
        A_Wq.reshape(D // 2, 2, H, Dh),
        A_Wk.reshape(D // 2, 2, H, Dh),
        A_Wv.reshape(D // 2, 2, H, Dh),
        A_Wo.reshape(H * Dh, D),
        B_w_r,
        B_w_gate,
        B_w_up,
        B_w_down,
    )
    return out.reshape(B, S, D)
```

```python
import contextlib
import functools


SCOPES = 0
UNROLL = 2
SCHED_F = [2,6,22]
SCHED_A = [2,6,16]
SCHED_M = [3,6,24]
SCHED_B = [3,5,24]
SCHED_L = [2,6,16]
CHAIN = 1
NX = 2
PLAN_X = [(1, 0, 0), (1, 0, 0)]
GROUPS = [(1,), (1,), (2,), (2,), (4,), (3,), (3,)]
PLAN = [(2, 0, 0), (2, 0, 0), (4, 0, 0), (3, 0, 0), (2, 8, 0), (1, 8, 2), (0, 0, 14)]
FFN_AT = [32,33,34,35,38,39]

import jax
import jax.numpy as jnp
from jax import lax
import jax.experimental.pallas as pl
import jax.experimental.pallas.tpu as pltpu

F32 = jnp.float32
BF16 = jnp.bfloat16
U32 = jnp.uint32

TOP_K = 2
LN_EPS = 1e-05
MASK_VALUE = -1000000000.0
PRE = 8


def scope(n):
    return jax.named_scope(n) if SCOPES else contextlib.nullcontext()


def _rbf16(x):
    return x.astype(BF16).astype(F32)


def _dot(lhs, words):
    return jnp.dot(lhs, pltpu.bitcast(words, BF16), preferred_element_type=F32)


def _split_pair(w_ref, p):
    for r in range(0, w_ref.shape[1], 16):
        a = w_ref[2 * p, r:r + 16]
        b = w_ref[2 * p + 1, r:r + 16]
        w_ref[2 * p, r:r + 16] = (a & jnp.uint32(0xFFFF)) | (b << 16)
        w_ref[2 * p + 1, r:r + 16] = (a >> 16) | (b & jnp.uint32(0xFFFF0000))


def _start(copies):
    for cp in copies:
        cp.start()


def _wait(copies):
    for cp in copies:
        cp.wait()


def _kernel(x_hbm, mem0_hbm, wq_hbm, wk_hbm, wv_hbm, wo_hbm, wr_hbm, wg_hbm, wu_hbm, wd_hbm,
            out_hbm,
            xbuf, membuf, wrbuf, hall, wq, wk, wv, wo, qpre, kpre, obuf, outbuf, rbuf,
            wg, wu, wd, xsel, yacc, gu,
            sem_x, sem_in, sem_qk, sem_v, sem_o, sem_ffn, sem_out):
    n_seg, T, D = xbuf.shape
    M = membuf.shape[0]
    H, _, Dh = wq.shape
    L = M + T
    scale = Dh ** (-0.5)
    n_pair = H // 2

    wq32, wk32, wv32, wo32 = (r.bitcast(U32) for r in (wq_hbm, wk_hbm, wv_hbm, wo_hbm))

    def qk_copies(p):
        return [pltpu.make_async_copy(src.at[:, b, p, :], dst.at[2 * p + b], sem_qk.at[p])
                for src, dst in ((wq32, wq), (wk32, wk)) for b in range(2)]

    def v_copies(p):
        return [pltpu.make_async_copy(wv32.at[:, b, p, :], wv.at[2 * p + b], sem_v.at[p])
                for b in range(2)]

    issued = [0, 0, 0]
    cp_wo = []

    def issue(plan):
        for kind, copies in enumerate((qk_copies, v_copies)):
            for p in range(issued[kind], issued[kind] + plan[kind]):
                _start(copies(p))
        if plan[2]:
            rows = pl.ds(issued[2] * Dh, plan[2] * Dh)
            cp_wo.append(pltpu.make_async_copy(wo32.at[rows], wo.at[rows], sem_o.at[len(cp_wo)]))
            cp_wo[-1].start()
        for kind in range(3):
            issued[kind] += plan[kind]

    x_seg = n_seg // NX
    cp_xp = [pltpu.make_async_copy(x_hbm.at[c * x_seg:(c + 1) * x_seg, T - PRE:, :],
                                   xbuf.at[c * x_seg:(c + 1) * x_seg, T - PRE:, :], sem_x.at[c])
             for c in range(NX)]
    cp_small = [pltpu.make_async_copy(mem0_hbm, membuf, sem_in.at[0]),
                pltpu.make_async_copy(wr_hbm, wrbuf, sem_in.at[1])]

    def x_rest(s0, s1, sem):
        return pltpu.make_async_copy(x_hbm.at[s0:s1, :T - PRE, :], xbuf.at[s0:s1, :T - PRE, :], sem)

    half_seg = n_seg // 2
    cp_xa = [x_rest(0, 3, sem_in.at[2]), x_rest(half_seg + 1, half_seg + 2, sem_in.at[3])]
    cp_xb = [x_rest(3, half_seg + 1, sem_in.at[4]), x_rest(half_seg + 2, n_seg, sem_in.at[5])]
    cp_ffn = [pltpu.make_async_copy(src.bitcast(U32), dst, sem_ffn.at[n])
              for n, (src, dst) in enumerate(((wg_hbm, wg), (wu_hbm, wu), (wd_hbm, wd)))]

    def layernorm(s, r0, after=None):
        xs = xbuf[s, r0:r0 + 8, :].astype(F32)
        mean = jnp.mean(xs, axis=-1, keepdims=True)
        if after is not None and CHAIN:
            mean = jnp.maximum(mean, jnp.minimum(mean, jnp.where(after > 0, 1.0, 0.0)))
        cen = xs - mean
        var = jnp.mean(cen * cen, axis=-1, keepdims=True)
        den = _rbf16(jnp.sqrt(_rbf16(_rbf16(var) + LN_EPS)))
        xn = _rbf16(_rbf16(xs - _rbf16(mean)) / den)
        hall[s, M + r0:M + r0 + 8, :] = xn
        return xn

    def finish_segments(segs):
        lane = lax.broadcasted_iota(jnp.int32, (8, 128), 1)
        w_r = wrbuf[...].astype(F32).reshape(1, D)
        r = None
        for s in segs:
            for r0 in range(0, T, 8):
                xn = layernorm(s, r0, r) if r0 < T - PRE else hall[s, M + r0:M + r0 + 8, :]
                r = _rbf16(jnp.sum(xn * w_r, axis=-1, keepdims=True))
                rbuf[r0:r0 + 8, :] = jnp.where(lane == s, r, rbuf[r0:r0 + 8, :])

    cp_xp[0].start()
    _start(cp_small)
    if NX > 1:
        cp_xp[1].start()
    for c in range(NX):
        with scope("waitx"):
            cp_xp[c].wait()
        if c + 2 < NX:
            cp_xp[c + 2].start()
        issue(PLAN_X[c])
        with scope("lnpre"):
            for s in range(c * x_seg, (c + 1) * x_seg):
                layernorm(s, T - PRE)

    _wait(cp_small)
    hall[0, :M, :] = membuf[...].astype(F32)
    rbuf[...] = jnp.full(rbuf.shape, -jnp.inf, F32)
    p0 = 0
    with scope("pairs"):
        for g, ((n_qk,), plan) in enumerate(zip(GROUPS, PLAN)):
            with scope("waitw"):
                for p in range(p0, p0 + n_qk):
                    _wait(qk_copies(p))
            with scope("waitissue"):
                issue(plan)
            if g == len(GROUPS) - 3:
                _start(cp_xa)
            if g == len(GROUPS) - 1:
                with scope("waitxa"):
                    _wait(cp_xa)
            with scope("grp"):
                for w_ref, pre in ((wq, qpre), (wk, kpre)):
                    for p in range(p0, p0 + n_qk):
                        _split_pair(w_ref, p)
                    for h in range(2 * p0, 2 * (p0 + n_qk)):
                        pre[h] = _dot(hall[:, L - PRE:, :].reshape(n_seg * PRE, D), w_ref[h])
                if p0 + n_qk == n_pair:
                    finish_segments([0])
            p0 += n_qk
    assert p0 == n_pair and issued == [n_pair] * 3
    with scope("ln0"):
        for p in range(n_pair):
            _wait(v_copies(p))

    def route():
        seg_id = lax.broadcasted_iota(jnp.int32, (T, 128), 1)
        tok = seg_id * T + lax.broadcasted_iota(jnp.int32, (T, 128), 0)
        r_all = rbuf[...]
        key = jnp.where(r_all != r_all, -jnp.inf, r_all)
        live = seg_id < n_seg
        sub = lax.broadcasted_iota(jnp.int32, (8, D), 0)
        x_sel = jnp.zeros((8, D), F32)
        idx, gate = [], []
        for n in range(TOP_K):
            best = jnp.max(jnp.where(live, key, -jnp.inf), keepdims=True)
            first = jnp.min(jnp.where(live & (key == best), tok, n_seg * T), keepdims=True)
            live = live & (tok != first)
            i = first[0, 0]
            x_sel = jnp.where(sub == n, hall[i // T, pl.ds(M + i % T, 1), :], x_sel)
            idx.append(i)
            gate.append(jax.nn.sigmoid(best))
        xsel[...] = x_sel
        yacc[...] = jnp.zeros(yacc.shape, F32)
        return idx, gate

    n_ffn = wg.shape[1] // 128

    def step(s, sched, ffn_slice=None, first=False, last=False):
        SK_S, SK_P, HA = sched
        q0 = M if last else 0
        ri = q0 + lax.broadcasted_iota(jnp.int32, (L - q0, L), 0)
        ci = lax.broadcasted_iota(jnp.int32, (L - q0, L), 1)
        mask = (ri < M) | (ri >= ci)
        pre_rows = pl.ds(pl.multiple_of(s * PRE, PRE), PRE)
        qkv, prob, act = {}, {}, []

        def project(h):
            if first and h % 2 == 0:
                _split_pair(wv, h // 2)
            k = _dot(hall[s, :L - PRE, :], wk[h])
            q = _dot(hall[s, :L - PRE, :], wq[h])
            v = _dot(hall[s], wv[h])
            q = jnp.concatenate([q, qpre[h, pre_rows, :]], axis=0)
            k = jnp.concatenate([k, kpre[h, pre_rows, :]], axis=0)
            qkv[h] = (q[q0:], k.astype(BF16), v.astype(BF16))

        def scores(h):
            q, k, _ = qkv[h]
            sc = lax.dot_general(q, k, (((1,), (1,)), ((), ())), preferred_element_type=F32)
            sc = jnp.where(mask, sc * scale, MASK_VALUE)
            e = jnp.exp(sc - jnp.max(sc, axis=-1, keepdims=True))
            prob[h] = e / jnp.sum(e, axis=-1, keepdims=True)

        def mix(h):
            obuf[q0:, h * Dh:(h + 1) * Dh] = jnp.dot(prob.pop(h), qkv.pop(h)[2],
                                                     preferred_element_type=F32)

        def out_proj(h0, h1, c0, c1):
            return _dot(obuf[q0:, h0 * Dh:h1 * Dh], wo[h0 * Dh // 2:h1 * Dh // 2, c0:c1])

        def ffn_piece(piece):
            t, slot, down = ffn_slice
            half = D // 2
            if piece == 0 and down:
                g = gu[slot, 0] + gu[slot, 1]
                act.append(g * jax.nn.sigmoid(g) * (gu[slot, 2] + gu[slot, 3]))
            if piece < 4:
                w_ref, k0 = (wg, wu)[piece // 2], piece % 2 * half
                cols = pl.ds(pl.multiple_of(jnp.minimum(t, n_ffn - 1) * 128, 128), 128)
                gu[slot, piece] = _dot(xsel[:, k0:k0 + half], w_ref[k0 // 2:(k0 + half) // 2, cols])
            elif down:
                c0 = piece % 2 * half
                rows = pl.ds(pl.multiple_of((t - UNROLL) * 64, 64), 64)
                yacc[:, c0:c0 + half] += _dot(act[0], wd[rows, c0:c0 + half])

        parts = []
        for i in range(H + D // 128):
            if i < H:
                project(i)
            else:
                if i == H and first:
                    with scope("waito"):
                        _wait(cp_wo)
                    _start(cp_xb)
                parts.append(out_proj(0, HA, (i - H) * 128, (i - H + 1) * 128))
            if ffn_slice is not None and i in FFN_AT:
                ffn_piece(FFN_AT.index(i))
            if 0 <= i - SK_S < H:
                scores(i - SK_S)
            if 0 <= i - SK_P < H:
                mix(i - SK_P)
        o = jnp.concatenate(parts, axis=1) + out_proj(HA, H, 0, D)

        if not last:
            hall[s + 1, :M, :] = o[:M]
        outbuf[s] = (xbuf[s].astype(F32) + o[M - q0:] + hall[s, M:, :]).astype(BF16)

    with scope("first"):
        step(0, SCHED_F, first=True)
        finish_segments([1])
        step(1, SCHED_F)
        finish_segments([2, half_seg + 1])
        _wait(cp_xb)
        _start(cp_ffn)

    s_last = n_seg - 2
    s_ffn = s_last - n_ffn - UNROLL
    assert s_ffn == half_seg and (s_ffn - 2) % UNROLL == 0 and n_ffn % UNROLL == 0

    def norm_steps(j, carry):
        for u in range(UNROLL):
            s = 2 + UNROLL * j + u
            step(s, SCHED_A)
            finish_segments([s + 1, s + half_seg])
        return carry

    def ffn_steps(j, carry):
        for u in range(UNROLL):
            step(s_ffn + UNROLL * j + u, SCHED_B, ffn_slice=(UNROLL * j + u, u, True))
        return carry

    with scope("loop_a"):
        lax.fori_loop(0, (s_ffn - 2) // UNROLL, norm_steps, 0)
    with scope("route"):
        _wait(cp_ffn)
        idx, gate = route()
        for u in range(UNROLL):
            step(s_ffn + u, SCHED_M, ffn_slice=(u, u, False))
    with scope("loop_b"):
        lax.fori_loop(1, (s_last - s_ffn) // UNROLL, ffn_steps, 0)

    def write_out(s0, s1, sem):
        row = lax.broadcasted_iota(jnp.int32, (T, D), 0)
        for n, i in enumerate(idx):
            @pl.when((i >= s0 * T) & (i < s1 * T))
            def _():
                blk = outbuf[i // T].astype(F32)
                upd = yacc[n:n + 1, :] * gate[n]
                outbuf[i // T] = jnp.where(row == i % T, blk + upd, blk).astype(BF16)
        cp = pltpu.make_async_copy(outbuf.at[s0:s1], out_hbm.at[s0:s1], sem)
        cp.start()
        return cp

    with scope("last"):
        cp_head = write_out(0, s_last, sem_out.at[0])
        for s in range(s_last, n_seg):
            step(s, SCHED_L, last=s == n_seg - 1)
    with scope("fin"):
        _wait([cp_head, write_out(s_last, n_seg, sem_out.at[1])])


@functools.partial(jax.jit, static_argnames=("A_seg_len",))
def pallas_parallel_sum__memory_aug_recurrent_mem_tr__moe_arch_mod__prompt_kernel(
    A_x: jax.Array,
    A_mem0: jax.Array,
    A_Wq: jax.Array,
    A_Wk: jax.Array,
    A_Wv: jax.Array,
    A_Wo: jax.Array,
    A_seg_len: int,
    B_x: jax.Array,
    B_w_r: jax.Array,
    B_w_gate: jax.Array,
    B_w_up: jax.Array,
    B_w_down: jax.Array,
):
    del B_x
    B, S, D = A_x.shape
    _, H, Dh = A_Wq.shape
    M = A_mem0.shape[1]
    T = int(A_seg_len)
    F = B_w_gate.shape[1]
    L = M + T
    n_seg = S // T
    assert B == 1 and S % T == 0 and T % 16 == 0 and M % 8 == 0 and Dh == 128 and H % 2 == 0
    assert n_seg % (H // 2) == 0 and n_seg <= 128

    any_spec = pl.BlockSpec(memory_space=pl.ANY)
    out = pl.pallas_call(
        _kernel,
        out_shape=jax.ShapeDtypeStruct((n_seg, T, D), A_x.dtype),
        in_specs=[any_spec] * 10,
        out_specs=any_spec,
        scratch_shapes=[
            pltpu.VMEM((n_seg, T, D), BF16),
            pltpu.VMEM((M, D), BF16),
            pltpu.VMEM((D,), BF16),
            pltpu.VMEM((n_seg, L, D), F32),
            pltpu.VMEM((H, D // 2, Dh), U32),
            pltpu.VMEM((H, D // 2, Dh), U32),
            pltpu.VMEM((H, D // 2, Dh), U32),
            pltpu.VMEM((H * Dh // 2, D), U32),
            pltpu.VMEM((H, n_seg * PRE, Dh), F32),
            pltpu.VMEM((H, n_seg * PRE, Dh), F32),
            pltpu.VMEM((L, H * Dh), F32),
            pltpu.VMEM((n_seg, T, D), BF16),
            pltpu.VMEM((T, 128), F32),
            pltpu.VMEM((D // 2, F), U32),
            pltpu.VMEM((D // 2, F), U32),
            pltpu.VMEM((F // 2, D), U32),
            pltpu.VMEM((8, D), F32),
            pltpu.VMEM((8, D), F32),
            pltpu.VMEM((UNROLL, 4, 8, 128), F32),
            pltpu.SemaphoreType.DMA((NX,)),
            pltpu.SemaphoreType.DMA((6,)),
            pltpu.SemaphoreType.DMA((H // 2,)),
            pltpu.SemaphoreType.DMA((H // 2,)),
            pltpu.SemaphoreType.DMA((H // 2,)),
            pltpu.SemaphoreType.DMA((3,)),
            pltpu.SemaphoreType.DMA((2,)),
        ],
        compiler_params=pltpu.CompilerParams(vmem_limit_bytes=120 * 1024 * 1024),
        name="rmt_mod_fused",
    )(
        A_x.reshape(n_seg, T, D),
        A_mem0.reshape(M, D),
        A_Wq.reshape(D // 2, 2, H, Dh),
        A_Wk.reshape(D // 2, 2, H, Dh),
        A_Wv.reshape(D // 2, 2, H, Dh),
        A_Wo.reshape(H * Dh, D),
        B_w_r,
        B_w_gate,
        B_w_up,
        B_w_down,
    )
    return out.reshape(B, S, D)
```

```python
import contextlib
import functools


SCOPES = 0
UNROLL = 2
SCHED_F = [2,6,22]
SCHED_A = [2,6,16]
SCHED_M = [3,6,24]
SCHED_B = [3,5,24]
SCHED_L = [2,6,16]
CHAIN = 1
NX = 2
PLAN_X = [(1, 0, 0), (1, 0, 0)]
GROUPS = [(1,), (1,), (2,), (4,), (4,), (8,), (12,)]
PLAN = [(2, 0, 0), (4, 0, 0), (4, 0, 0), (8, 0, 0), (8, 0, 0), (4, 6, 0), (0, 10, 16)]
FFN_AT = [32,33,34,35,38,39]

import jax
import jax.numpy as jnp
from jax import lax
import jax.experimental.pallas as pl
import jax.experimental.pallas.tpu as pltpu

F32 = jnp.float32
BF16 = jnp.bfloat16
U32 = jnp.uint32

TOP_K = 2
LN_EPS = 1e-05
MASK_VALUE = -1000000000.0
PRE = 8


def scope(n):
    return jax.named_scope(n) if SCOPES else contextlib.nullcontext()


def _rbf16(x):
    return x.astype(BF16).astype(F32)


def _dot(lhs, words):
    return jnp.dot(lhs, pltpu.bitcast(words, BF16), preferred_element_type=F32)


def _split_pair(w_ref, p):
    for r in range(0, w_ref.shape[1], 16):
        a = w_ref[2 * p, r:r + 16]
        b = w_ref[2 * p + 1, r:r + 16]
        w_ref[2 * p, r:r + 16] = (a & jnp.uint32(0xFFFF)) | (b << 16)
        w_ref[2 * p + 1, r:r + 16] = (a >> 16) | (b & jnp.uint32(0xFFFF0000))


def _start(copies):
    for cp in copies:
        cp.start()


def _wait(copies):
    for cp in copies:
        cp.wait()


def _kernel(x_hbm, mem0_hbm, wq_hbm, wk_hbm, wv_hbm, wo_hbm, wr_hbm, wg_hbm, wu_hbm, wd_hbm,
            out_hbm,
            xbuf, membuf, wrbuf, hall, wq, wk, wv, wo, qpre, kpre, obuf, outbuf, rbuf,
            wg, wu, wd, xsel, yacc, gu,
            sem_x, sem_in, sem_qk, sem_v, sem_o, sem_ffn, sem_out):
    n_seg, T, D = xbuf.shape
    M = membuf.shape[0]
    H, _, Dh = wq.shape
    L = M + T
    scale = Dh ** (-0.5)
    n_pair = H // 2

    wq32, wk32, wv32, wo32 = (r.bitcast(U32) for r in (wq_hbm, wk_hbm, wv_hbm, wo_hbm))

    def qk_copies(j):
        src, dst = ((wq32, wq), (wk32, wk))[j % 2]
        return [pltpu.make_async_copy(src.at[:, b, j // 2, :], dst.at[j // 2 * 2 + b], sem_qk.at[j])
                for b in range(2)]

    def v_copies(p):
        return [pltpu.make_async_copy(wv32.at[:, b, p, :], wv.at[2 * p + b], sem_v.at[p])
                for b in range(2)]

    issued = [0, 0, 0]
    cp_wo = []

    def issue(plan):
        for kind, copies in enumerate((qk_copies, v_copies)):
            for p in range(issued[kind], issued[kind] + plan[kind]):
                _start(copies(p))
        if plan[2]:
            rows = pl.ds(issued[2] * Dh, plan[2] * Dh)
            cp_wo.append(pltpu.make_async_copy(wo32.at[rows], wo.at[rows], sem_o.at[len(cp_wo)]))
            cp_wo[-1].start()
        for kind in range(3):
            issued[kind] += plan[kind]

    x_seg = n_seg // NX
    cp_xp = [pltpu.make_async_copy(x_hbm.at[c * x_seg:(c + 1) * x_seg, T - PRE:, :],
                                   xbuf.at[c * x_seg:(c + 1) * x_seg, T - PRE:, :], sem_x.at[c])
             for c in range(NX)]
    cp_small = [pltpu.make_async_copy(mem0_hbm, membuf, sem_in.at[0]),
                pltpu.make_async_copy(wr_hbm, wrbuf, sem_in.at[1])]

    def x_rest(s0, s1, sem):
        return pltpu.make_async_copy(x_hbm.at[s0:s1, :T - PRE, :], xbuf.at[s0:s1, :T - PRE, :], sem)

    half_seg = n_seg // 2
    cp_xa = [x_rest(0, 3, sem_in.at[2]), x_rest(half_seg + 1, half_seg + 2, sem_in.at[3])]
    cp_xb = [x_rest(3, half_seg + 1, sem_in.at[4]), x_rest(half_seg + 2, n_seg, sem_in.at[5])]
    cp_ffn = [pltpu.make_async_copy(src.bitcast(U32), dst, sem_ffn.at[n])
              for n, (src, dst) in enumerate(((wg_hbm, wg), (wu_hbm, wu), (wd_hbm, wd)))]

    def layernorm(s, r0, after=None):
        xs = xbuf[s, r0:r0 + 8, :].astype(F32)
        mean = jnp.mean(xs, axis=-1, keepdims=True)
        if after is not None and CHAIN:
            mean = jnp.maximum(mean, jnp.minimum(mean, jnp.where(after > 0, 1.0, 0.0)))
        cen = xs - mean
        var = jnp.mean(cen * cen, axis=-1, keepdims=True)
        den = _rbf16(jnp.sqrt(_rbf16(_rbf16(var) + LN_EPS)))
        xn = _rbf16(_rbf16(xs - _rbf16(mean)) / den)
        hall[s, M + r0:M + r0 + 8, :] = xn
        return xn

    def finish_segments(segs):
        lane = lax.broadcasted_iota(jnp.int32, (8, 128), 1)
        w_r = wrbuf[...].astype(F32).reshape(1, D)
        r = None
        for s in segs:
            for r0 in range(0, T, 8):
                xn = layernorm(s, r0, r) if r0 < T - PRE else hall[s, M + r0:M + r0 + 8, :]
                r = _rbf16(jnp.sum(xn * w_r, axis=-1, keepdims=True))
                rbuf[r0:r0 + 8, :] = jnp.where(lane == s, r, rbuf[r0:r0 + 8, :])

    cp_xp[0].start()
    _start(cp_small)
    if NX > 1:
        cp_xp[1].start()
    for c in range(NX):
        with scope("waitx"):
            cp_xp[c].wait()
        if c + 2 < NX:
            cp_xp[c + 2].start()
        issue(PLAN_X[c])
        with scope("lnpre"):
            for s in range(c * x_seg, (c + 1) * x_seg):
                layernorm(s, T - PRE)

    _wait(cp_small)
    hall[0, :M, :] = membuf[...].astype(F32)
    rbuf[...] = jnp.full(rbuf.shape, -jnp.inf, F32)
    j0 = 0
    with scope("pairs"):
        for g, ((n_job,), plan) in enumerate(zip(GROUPS, PLAN)):
            with scope("waitw"):
                for j in range(j0, j0 + n_job):
                    _wait(qk_copies(j))
            with scope("waitissue"):
                issue(plan)
            if g == len(GROUPS) - 3:
                _start(cp_xa)
            if g == len(GROUPS) - 1:
                with scope("waitxa"):
                    _wait(cp_xa)
            with scope("grp"):
                for j in range(j0, j0 + n_job):
                    w_ref, pre = ((wq, qpre), (wk, kpre))[j % 2]
                    _split_pair(w_ref, j // 2)
                    for h in range(j // 2 * 2, j // 2 * 2 + 2):
                        pre[h] = _dot(hall[:, L - PRE:, :].reshape(n_seg * PRE, D), w_ref[h])
                if g == len(GROUPS) - 1:
                    finish_segments([0])
            j0 += n_job
    assert j0 == H and issued == [H, n_pair, n_pair]
    with scope("ln0"):
        for p in range(n_pair):
            _wait(v_copies(p))

    def route():
        seg_id = lax.broadcasted_iota(jnp.int32, (T, 128), 1)
        tok = seg_id * T + lax.broadcasted_iota(jnp.int32, (T, 128), 0)
        r_all = rbuf[...]
        key = jnp.where(r_all != r_all, -jnp.inf, r_all)
        live = seg_id < n_seg
        sub = lax.broadcasted_iota(jnp.int32, (8, D), 0)
        x_sel = jnp.zeros((8, D), F32)
        idx, gate = [], []
        for n in range(TOP_K):
            best = jnp.max(jnp.where(live, key, -jnp.inf), keepdims=True)
            first = jnp.min(jnp.where(live & (key == best), tok, n_seg * T), keepdims=True)
            live = live & (tok != first)
            i = first[0, 0]
            x_sel = jnp.where(sub == n, hall[i // T, pl.ds(M + i % T, 1), :], x_sel)
            idx.append(i)
            gate.append(jax.nn.sigmoid(best))
        xsel[...] = x_sel
        yacc[...] = jnp.zeros(yacc.shape, F32)
        return idx, gate

    n_ffn = wg.shape[1] // 128

    def step(s, sched, ffn_slice=None, first=False, last=False):
        SK_S, SK_P, HA = sched
        q0 = M if last else 0
        ri = q0 + lax.broadcasted_iota(jnp.int32, (L - q0, L), 0)
        ci = lax.broadcasted_iota(jnp.int32, (L - q0, L), 1)
        mask = (ri < M) | (ri >= ci)
        pre_rows = pl.ds(pl.multiple_of(s * PRE, PRE), PRE)
        qkv, prob, act = {}, {}, []

        def project(h):
            if first and h % 2 == 0:
                _split_pair(wv, h // 2)
            k = _dot(hall[s, :L - PRE, :], wk[h])
            q = _dot(hall[s, :L - PRE, :], wq[h])
            v = _dot(hall[s], wv[h])
            q = jnp.concatenate([q, qpre[h, pre_rows, :]], axis=0)
            k = jnp.concatenate([k, kpre[h, pre_rows, :]], axis=0)
            qkv[h] = (q[q0:], k.astype(BF16), v.astype(BF16))

        def scores(h):
            q, k, _ = qkv[h]
            sc = lax.dot_general(q, k, (((1,), (1,)), ((), ())), preferred_element_type=F32)
            sc = jnp.where(mask, sc * scale, MASK_VALUE)
            e = jnp.exp(sc - jnp.max(sc, axis=-1, keepdims=True))
            prob[h] = e / jnp.sum(e, axis=-1, keepdims=True)

        def mix(h):
            obuf[q0:, h * Dh:(h + 1) * Dh] = jnp.dot(prob.pop(h), qkv.pop(h)[2],
                                                     preferred_element_type=F32)

        def out_proj(h0, h1, c0, c1):
            return _dot(obuf[q0:, h0 * Dh:h1 * Dh], wo[h0 * Dh // 2:h1 * Dh // 2, c0:c1])

        def ffn_piece(piece):
            t, slot, down = ffn_slice
            half = D // 2
            if piece == 0 and down:
                g = gu[slot, 0] + gu[slot, 1]
                act.append(g * jax.nn.sigmoid(g) * (gu[slot, 2] + gu[slot, 3]))
            if piece < 4:
                w_ref, k0 = (wg, wu)[piece // 2], piece % 2 * half
                cols = pl.ds(pl.multiple_of(jnp.minimum(t, n_ffn - 1) * 128, 128), 128)
                gu[slot, piece] = _dot(xsel[:, k0:k0 + half], w_ref[k0 // 2:(k0 + half) // 2, cols])
            elif down:
                c0 = piece % 2 * half
                rows = pl.ds(pl.multiple_of((t - UNROLL) * 64, 64), 64)
                yacc[:, c0:c0 + half] += _dot(act[0], wd[rows, c0:c0 + half])

        parts = []
        for i in range(H + D // 128):
            if i < H:
                project(i)
            else:
                if i == H and first:
                    with scope("waito"):
                        _wait(cp_wo)
                    _start(cp_xb)
                parts.append(out_proj(0, HA, (i - H) * 128, (i - H + 1) * 128))
            if ffn_slice is not None and i in FFN_AT:
                ffn_piece(FFN_AT.index(i))
            if 0 <= i - SK_S < H:
                scores(i - SK_S)
            if 0 <= i - SK_P < H:
                mix(i - SK_P)
        o = jnp.concatenate(parts, axis=1) + out_proj(HA, H, 0, D)

        if not last:
            hall[s + 1, :M, :] = o[:M]
        outbuf[s] = (xbuf[s].astype(F32) + o[M - q0:] + hall[s, M:, :]).astype(BF16)

    with scope("first"):
        step(0, SCHED_F, first=True)
        finish_segments([1])
        step(1, SCHED_F)
        finish_segments([2, half_seg + 1])
        _wait(cp_xb)
        _start(cp_ffn)

    s_last = n_seg - 2
    s_ffn = s_last - n_ffn - UNROLL
    assert s_ffn == half_seg and (s_ffn - 2) % UNROLL == 0 and n_ffn % UNROLL == 0

    def norm_steps(j, carry):
        for u in range(UNROLL):
            s = 2 + UNROLL * j + u
            step(s, SCHED_A)
            finish_segments([s + 1, s + half_seg])
        return carry

    def ffn_steps(j, carry):
        for u in range(UNROLL):
            step(s_ffn + UNROLL * j + u, SCHED_B, ffn_slice=(UNROLL * j + u, u, True))
        return carry

    with scope("loop_a"):
        lax.fori_loop(0, (s_ffn - 2) // UNROLL, norm_steps, 0)
    with scope("route"):
        _wait(cp_ffn)
        idx, gate = route()
        for u in range(UNROLL):
            step(s_ffn + u, SCHED_M, ffn_slice=(u, u, False))
    with scope("loop_b"):
        lax.fori_loop(1, (s_last - s_ffn) // UNROLL, ffn_steps, 0)

    def write_out(s0, s1, sem):
        row = lax.broadcasted_iota(jnp.int32, (T, D), 0)
        for n, i in enumerate(idx):
            @pl.when((i >= s0 * T) & (i < s1 * T))
            def _():
                blk = outbuf[i // T].astype(F32)
                upd = yacc[n:n + 1, :] * gate[n]
                outbuf[i // T] = jnp.where(row == i % T, blk + upd, blk).astype(BF16)
        cp = pltpu.make_async_copy(outbuf.at[s0:s1], out_hbm.at[s0:s1], sem)
        cp.start()
        return cp

    with scope("last"):
        cp_head = write_out(0, s_last, sem_out.at[0])
        for s in range(s_last, n_seg):
            step(s, SCHED_L, last=s == n_seg - 1)
    with scope("fin"):
        _wait([cp_head, write_out(s_last, n_seg, sem_out.at[1])])


@functools.partial(jax.jit, static_argnames=("A_seg_len",))
def pallas_parallel_sum__memory_aug_recurrent_mem_tr__moe_arch_mod__prompt_kernel(
    A_x: jax.Array,
    A_mem0: jax.Array,
    A_Wq: jax.Array,
    A_Wk: jax.Array,
    A_Wv: jax.Array,
    A_Wo: jax.Array,
    A_seg_len: int,
    B_x: jax.Array,
    B_w_r: jax.Array,
    B_w_gate: jax.Array,
    B_w_up: jax.Array,
    B_w_down: jax.Array,
):
    del B_x
    B, S, D = A_x.shape
    _, H, Dh = A_Wq.shape
    M = A_mem0.shape[1]
    T = int(A_seg_len)
    F = B_w_gate.shape[1]
    L = M + T
    n_seg = S // T
    assert B == 1 and S % T == 0 and T % 16 == 0 and M % 8 == 0 and Dh == 128 and H % 2 == 0
    assert n_seg % (H // 2) == 0 and n_seg <= 128

    any_spec = pl.BlockSpec(memory_space=pl.ANY)
    out = pl.pallas_call(
        _kernel,
        out_shape=jax.ShapeDtypeStruct((n_seg, T, D), A_x.dtype),
        in_specs=[any_spec] * 10,
        out_specs=any_spec,
        scratch_shapes=[
            pltpu.VMEM((n_seg, T, D), BF16),
            pltpu.VMEM((M, D), BF16),
            pltpu.VMEM((D,), BF16),
            pltpu.VMEM((n_seg, L, D), F32),
            pltpu.VMEM((H, D // 2, Dh), U32),
            pltpu.VMEM((H, D // 2, Dh), U32),
            pltpu.VMEM((H, D // 2, Dh), U32),
            pltpu.VMEM((H * Dh // 2, D), U32),
            pltpu.VMEM((H, n_seg * PRE, Dh), F32),
            pltpu.VMEM((H, n_seg * PRE, Dh), F32),
            pltpu.VMEM((L, H * Dh), F32),
            pltpu.VMEM((n_seg, T, D), BF16),
            pltpu.VMEM((T, 128), F32),
            pltpu.VMEM((D // 2, F), U32),
            pltpu.VMEM((D // 2, F), U32),
            pltpu.VMEM((F // 2, D), U32),
            pltpu.VMEM((8, D), F32),
            pltpu.VMEM((8, D), F32),
            pltpu.VMEM((UNROLL, 4, 8, 128), F32),
            pltpu.SemaphoreType.DMA((NX,)),
            pltpu.SemaphoreType.DMA((6,)),
            pltpu.SemaphoreType.DMA((H,)),
            pltpu.SemaphoreType.DMA((H // 2,)),
            pltpu.SemaphoreType.DMA((H // 2,)),
            pltpu.SemaphoreType.DMA((3,)),
            pltpu.SemaphoreType.DMA((2,)),
        ],
        compiler_params=pltpu.CompilerParams(vmem_limit_bytes=120 * 1024 * 1024),
        name="rmt_mod_fused",
    )(
        A_x.reshape(n_seg, T, D),
        A_mem0.reshape(M, D),
        A_Wq.reshape(D // 2, 2, H, Dh),
        A_Wk.reshape(D // 2, 2, H, Dh),
        A_Wv.reshape(D // 2, 2, H, Dh),
        A_Wo.reshape(H * Dh, D),
        B_w_r,
        B_w_gate,
        B_w_up,
        B_w_down,
    )
    return out.reshape(B, S, D)
```

```python
import contextlib
import functools


SCOPES = 0
UNROLL = 2
SCHED_F = [2,6,16,1,1]
SCHED_A = [2,6,16,1,1]
SCHED_M = [1,5,24,1,2]
SCHED_B = [1,5,24,1,2]
SCHED_L = [2,6,16,1,1]
CHAIN = 1
NX = 2
PLAN_X = [(1, 0, 0), (1, 0, 0)]
GROUPS = [(1,), (1,), (2,), (4,), (4,), (8,), (12,)]
PLAN = [(2, 0, 0), (4, 0, 0), (4, 0, 0), (8, 0, 0), (8, 0, 0), (4, 6, 0), (0, 10, 16)]
FFN_AT = [32,33,34,35,38,39]

import jax
import jax.numpy as jnp
from jax import lax
import jax.experimental.pallas as pl
import jax.experimental.pallas.tpu as pltpu

F32 = jnp.float32
BF16 = jnp.bfloat16
U32 = jnp.uint32

TOP_K = 2
LN_EPS = 1e-05
MASK_VALUE = -1000000000.0
PRE = 8


def scope(n):
    return jax.named_scope(n) if SCOPES else contextlib.nullcontext()


def _rbf16(x):
    return x.astype(BF16).astype(F32)


def _dot(lhs, words):
    return jnp.dot(lhs, pltpu.bitcast(words, BF16), preferred_element_type=F32)


def _split_pair(w_ref, p):
    for r in range(0, w_ref.shape[1], 16):
        a = w_ref[2 * p, r:r + 16]
        b = w_ref[2 * p + 1, r:r + 16]
        w_ref[2 * p, r:r + 16] = (a & jnp.uint32(0xFFFF)) | (b << 16)
        w_ref[2 * p + 1, r:r + 16] = (a >> 16) | (b & jnp.uint32(0xFFFF0000))


def _start(copies):
    for cp in copies:
        cp.start()


def _wait(copies):
    for cp in copies:
        cp.wait()


def _kernel(x_hbm, mem0_hbm, wq_hbm, wk_hbm, wv_hbm, wo_hbm, wr_hbm, wg_hbm, wu_hbm, wd_hbm,
            out_hbm,
            xbuf, membuf, wrbuf, hall, wq, wk, wv, wo, qpre, kpre, obuf, outbuf, rbuf,
            wg, wu, wd, xsel, yacc, gu,
            sem_x, sem_in, sem_qk, sem_v, sem_o, sem_ffn, sem_out):
    n_seg, T, D = xbuf.shape
    M = membuf.shape[0]
    H, _, Dh = wq.shape
    L = M + T
    scale = Dh ** (-0.5)
    n_pair = H // 2

    wq32, wk32, wv32, wo32 = (r.bitcast(U32) for r in (wq_hbm, wk_hbm, wv_hbm, wo_hbm))

    def qk_copies(j):
        src, dst = ((wq32, wq), (wk32, wk))[j % 2]
        return [pltpu.make_async_copy(src.at[:, b, j // 2, :], dst.at[j // 2 * 2 + b], sem_qk.at[j])
                for b in range(2)]

    def v_copies(p):
        return [pltpu.make_async_copy(wv32.at[:, b, p, :], wv.at[2 * p + b], sem_v.at[p])
                for b in range(2)]

    issued = [0, 0, 0]
    cp_wo = []

    def issue(plan):
        for kind, copies in enumerate((qk_copies, v_copies)):
            for p in range(issued[kind], issued[kind] + plan[kind]):
                _start(copies(p))
        if plan[2]:
            rows = pl.ds(issued[2] * Dh, plan[2] * Dh)
            cp_wo.append(pltpu.make_async_copy(wo32.at[rows], wo.at[rows], sem_o.at[len(cp_wo)]))
            cp_wo[-1].start()
        for kind in range(3):
            issued[kind] += plan[kind]

    x_seg = n_seg // NX
    cp_xp = [pltpu.make_async_copy(x_hbm.at[c * x_seg:(c + 1) * x_seg, T - PRE:, :],
                                   xbuf.at[c * x_seg:(c + 1) * x_seg, T - PRE:, :], sem_x.at[c])
             for c in range(NX)]
    cp_small = [pltpu.make_async_copy(mem0_hbm, membuf, sem_in.at[0]),
                pltpu.make_async_copy(wr_hbm, wrbuf, sem_in.at[1])]

    def x_rest(s0, s1, sem):
        return pltpu.make_async_copy(x_hbm.at[s0:s1, :T - PRE, :], xbuf.at[s0:s1, :T - PRE, :], sem)

    half_seg = n_seg // 2
    cp_xa = [x_rest(0, 3, sem_in.at[2]), x_rest(half_seg + 1, half_seg + 2, sem_in.at[3])]
    cp_xb = [x_rest(3, half_seg + 1, sem_in.at[4]), x_rest(half_seg + 2, n_seg, sem_in.at[5])]
    cp_ffn = [pltpu.make_async_copy(src.bitcast(U32), dst, sem_ffn.at[n])
              for n, (src, dst) in enumerate(((wg_hbm, wg), (wu_hbm, wu), (wd_hbm, wd)))]

    def layernorm(s, r0, after=None):
        xs = xbuf[s, r0:r0 + 8, :].astype(F32)
        mean = jnp.mean(xs, axis=-1, keepdims=True)
        if after is not None and CHAIN:
            mean = jnp.maximum(mean, jnp.minimum(mean, jnp.where(after > 0, 1.0, 0.0)))
        cen = xs - mean
        var = jnp.mean(cen * cen, axis=-1, keepdims=True)
        den = _rbf16(jnp.sqrt(_rbf16(_rbf16(var) + LN_EPS)))
        xn = _rbf16(_rbf16(xs - _rbf16(mean)) / den)
        hall[s, M + r0:M + r0 + 8, :] = xn
        return xn

    def finish_segments(segs):
        lane = lax.broadcasted_iota(jnp.int32, (8, 128), 1)
        w_r = wrbuf[...].astype(F32).reshape(1, D)
        r = None
        for s in segs:
            for r0 in range(0, T, 8):
                xn = layernorm(s, r0, r) if r0 < T - PRE else hall[s, M + r0:M + r0 + 8, :]
                r = _rbf16(jnp.sum(xn * w_r, axis=-1, keepdims=True))
                rbuf[r0:r0 + 8, :] = jnp.where(lane == s, r, rbuf[r0:r0 + 8, :])

    cp_xp[0].start()
    _start(cp_small)
    if NX > 1:
        cp_xp[1].start()
    for c in range(NX):
        with scope("waitx"):
            cp_xp[c].wait()
        if c + 2 < NX:
            cp_xp[c + 2].start()
        issue(PLAN_X[c])
        with scope("lnpre"):
            for s in range(c * x_seg, (c + 1) * x_seg):
                layernorm(s, T - PRE)

    _wait(cp_small)
    hall[0, :M, :] = membuf[...].astype(F32)
    rbuf[...] = jnp.full(rbuf.shape, -jnp.inf, F32)
    j0 = 0
    with scope("pairs"):
        for g, ((n_job,), plan) in enumerate(zip(GROUPS, PLAN)):
            with scope("waitw"):
                for j in range(j0, j0 + n_job):
                    _wait(qk_copies(j))
            with scope("waitissue"):
                issue(plan)
            if g == len(GROUPS) - 3:
                _start(cp_xa)
            if g == len(GROUPS) - 1:
                with scope("waitxa"):
                    _wait(cp_xa)
            with scope("grp"):
                for j in range(j0, j0 + n_job):
                    w_ref, pre = ((wq, qpre), (wk, kpre))[j % 2]
                    _split_pair(w_ref, j // 2)
                    for h in range(j // 2 * 2, j // 2 * 2 + 2):
                        pre[h] = _dot(hall[:, L - PRE:, :].reshape(n_seg * PRE, D), w_ref[h])
                if g == len(GROUPS) - 1:
                    finish_segments([0])
            j0 += n_job
    assert j0 == H and issued == [H, n_pair, n_pair]
    with scope("ln0"):
        for p in range(n_pair):
            _wait(v_copies(p))

    def route():
        seg_id = lax.broadcasted_iota(jnp.int32, (T, 128), 1)
        tok = seg_id * T + lax.broadcasted_iota(jnp.int32, (T, 128), 0)
        r_all = rbuf[...]
        key = jnp.where(r_all != r_all, -jnp.inf, r_all)
        live = seg_id < n_seg
        sub = lax.broadcasted_iota(jnp.int32, (8, D), 0)
        x_sel = jnp.zeros((8, D), F32)
        idx, gate = [], []
        for n in range(TOP_K):
            best = jnp.max(jnp.where(live, key, -jnp.inf), keepdims=True)
            first = jnp.min(jnp.where(live & (key == best), tok, n_seg * T), keepdims=True)
            live = live & (tok != first)
            i = first[0, 0]
            x_sel = jnp.where(sub == n, hall[i // T, pl.ds(M + i % T, 1), :], x_sel)
            idx.append(i)
            gate.append(jax.nn.sigmoid(best))
        xsel[...] = x_sel
        yacc[...] = jnp.zeros(yacc.shape, F32)
        return idx, gate

    n_ffn = wg.shape[1] // 128

    def step(s, sched, ffn_slice=None, first=False, last=False):
        SK_S, SK_P, HA, KSPLIT, ROT = sched
        q0 = M if last else 0
        ri = q0 + lax.broadcasted_iota(jnp.int32, (L - q0, L), 0)
        ci = lax.broadcasted_iota(jnp.int32, (L - q0, L), 1)
        mask = (ri < M) | (ri >= ci)
        pre_rows = pl.ds(pl.multiple_of(s * PRE, PRE), PRE)
        qkv, prob, act = {}, {}, []

        def project(h):
            if first and h % 2 == 0:
                _split_pair(wv, h // 2)
            if h == 0 and KSPLIT:
                def half(n):
                    d, w = slice(n * D // 2, (n + 1) * D // 2), slice(n * D // 4, (n + 1) * D // 4)
                    return (_dot(hall[s, :L - PRE, d], wk[h, w]),
                            _dot(hall[s, :L - PRE, d], wq[h, w]), _dot(hall[s, :, d], wv[h, w]))
                k, q, v = (a + b for a, b in zip(half(0), half(1)))
            else:
                k = _dot(hall[s, :L - PRE, :], wk[h])
                q = _dot(hall[s, :L - PRE, :], wq[h])
                v = _dot(hall[s], wv[h])
            q = jnp.concatenate([q, qpre[h, pre_rows, :]], axis=0)
            k = jnp.concatenate([k, kpre[h, pre_rows, :]], axis=0)
            qkv[h] = (q[q0:], k.astype(BF16), v.astype(BF16))

        def scores(h):
            q, k, _ = qkv[h]
            sc = lax.dot_general(q, k, (((1,), (1,)), ((), ())), preferred_element_type=F32)
            sc = jnp.where(mask, sc * scale, MASK_VALUE)
            e = jnp.exp(sc - jnp.max(sc, axis=-1, keepdims=True))
            prob[h] = e / jnp.sum(e, axis=-1, keepdims=True)

        def mix(h):
            obuf[q0:, h * Dh:(h + 1) * Dh] = jnp.dot(prob.pop(h), qkv.pop(h)[2],
                                                     preferred_element_type=F32)

        def out_proj(h0, h1, c0, c1):
            return _dot(obuf[q0:, h0 * Dh:h1 * Dh], wo[h0 * Dh // 2:h1 * Dh // 2, c0:c1])

        def ffn_piece(piece):
            t, slot, down = ffn_slice
            half = D // 2
            if piece == 0 and down:
                g = gu[slot, 0] + gu[slot, 1]
                act.append(g * jax.nn.sigmoid(g) * (gu[slot, 2] + gu[slot, 3]))
            if piece < 4:
                w_ref, k0 = (wg, wu)[piece // 2], piece % 2 * half
                cols = pl.ds(pl.multiple_of(jnp.minimum(t, n_ffn - 1) * 128, 128), 128)
                gu[slot, piece] = _dot(xsel[:, k0:k0 + half], w_ref[k0 // 2:(k0 + half) // 2, cols])
            elif down:
                c0 = piece % 2 * half
                rows = pl.ds(pl.multiple_of((t - UNROLL) * 64, 64), 64)
                yacc[:, c0:c0 + half] += _dot(act[0], wd[rows, c0:c0 + half])

        parts = []
        for i in range(H + D // 128):
            if i < H:
                project(i)
            else:
                if i == H and first:
                    with scope("waito"):
                        _wait(cp_wo)
                    _start(cp_xb)
                parts.append(out_proj(0, HA, (i - H) * 128, (i - H + 1) * 128))
            if ffn_slice is not None and i in FFN_AT:
                ffn_piece(FFN_AT.index(i))
            if 0 <= i - SK_S < H:
                scores(i - SK_S)
            if 0 <= i - SK_P < H:
                mix(i - SK_P)
        if ROT == 0:
            o = jnp.concatenate(parts, axis=1) + out_proj(HA, H, 0, D)
        else:
            hi = jnp.concatenate(parts[ROT:], axis=1) + out_proj(HA, H, ROT * 128, D)
            lo = jnp.concatenate(parts[:ROT], axis=1) + out_proj(HA, H, 0, ROT * 128)
            o = jnp.concatenate([lo, hi], axis=1)

        if not last:
            hall[s + 1, :M, :] = o[:M]
        outbuf[s] = (xbuf[s].astype(F32) + o[M - q0:] + hall[s, M:, :]).astype(BF16)

    with scope("first"):
        step(0, SCHED_F, first=True)
        finish_segments([1])
        step(1, SCHED_F)
        finish_segments([2, half_seg + 1])
        _wait(cp_xb)
        _start(cp_ffn)

    s_last = n_seg - 2
    s_ffn = s_last - n_ffn - UNROLL
    assert s_ffn == half_seg and (s_ffn - 2) % UNROLL == 0 and n_ffn % UNROLL == 0

    def norm_steps(j, carry):
        for u in range(UNROLL):
            s = 2 + UNROLL * j + u
            step(s, SCHED_A)
            finish_segments([s + 1, s + half_seg])
        return carry

    def ffn_steps(j, carry):
        for u in range(UNROLL):
            step(s_ffn + UNROLL * j + u, SCHED_B, ffn_slice=(UNROLL * j + u, u, True))
        return carry

    with scope("loop_a"):
        lax.fori_loop(0, (s_ffn - 2) // UNROLL, norm_steps, 0)
    with scope("route"):
        _wait(cp_ffn)
        idx, gate = route()
        for u in range(UNROLL):
            step(s_ffn + u, SCHED_M, ffn_slice=(u, u, False))
    with scope("loop_b"):
        lax.fori_loop(1, (s_last - s_ffn) // UNROLL, ffn_steps, 0)

    def write_out(s0, s1, sem):
        row = lax.broadcasted_iota(jnp.int32, (T, D), 0)
        for n, i in enumerate(idx):
            @pl.when((i >= s0 * T) & (i < s1 * T))
            def _():
                blk = outbuf[i // T].astype(F32)
                upd = yacc[n:n + 1, :] * gate[n]
                outbuf[i // T] = jnp.where(row == i % T, blk + upd, blk).astype(BF16)
        cp = pltpu.make_async_copy(outbuf.at[s0:s1], out_hbm.at[s0:s1], sem)
        cp.start()
        return cp

    with scope("last"):
        cp_head = write_out(0, s_last, sem_out.at[0])
        for s in range(s_last, n_seg):
            step(s, SCHED_L, last=s == n_seg - 1)
    with scope("fin"):
        _wait([cp_head, write_out(s_last, n_seg, sem_out.at[1])])


@functools.partial(jax.jit, static_argnames=("A_seg_len",))
def pallas_parallel_sum__memory_aug_recurrent_mem_tr__moe_arch_mod__prompt_kernel(
    A_x: jax.Array,
    A_mem0: jax.Array,
    A_Wq: jax.Array,
    A_Wk: jax.Array,
    A_Wv: jax.Array,
    A_Wo: jax.Array,
    A_seg_len: int,
    B_x: jax.Array,
    B_w_r: jax.Array,
    B_w_gate: jax.Array,
    B_w_up: jax.Array,
    B_w_down: jax.Array,
):
    del B_x
    B, S, D = A_x.shape
    _, H, Dh = A_Wq.shape
    M = A_mem0.shape[1]
    T = int(A_seg_len)
    F = B_w_gate.shape[1]
    L = M + T
    n_seg = S // T
    assert B == 1 and S % T == 0 and T % 16 == 0 and M % 8 == 0 and Dh == 128 and H % 2 == 0
    assert n_seg % (H // 2) == 0 and n_seg <= 128

    any_spec = pl.BlockSpec(memory_space=pl.ANY)
    out = pl.pallas_call(
        _kernel,
        out_shape=jax.ShapeDtypeStruct((n_seg, T, D), A_x.dtype),
        in_specs=[any_spec] * 10,
        out_specs=any_spec,
        scratch_shapes=[
            pltpu.VMEM((n_seg, T, D), BF16),
            pltpu.VMEM((M, D), BF16),
            pltpu.VMEM((D,), BF16),
            pltpu.VMEM((n_seg, L, D), F32),
            pltpu.VMEM((H, D // 2, Dh), U32),
            pltpu.VMEM((H, D // 2, Dh), U32),
            pltpu.VMEM((H, D // 2, Dh), U32),
            pltpu.VMEM((H * Dh // 2, D), U32),
            pltpu.VMEM((H, n_seg * PRE, Dh), F32),
            pltpu.VMEM((H, n_seg * PRE, Dh), F32),
            pltpu.VMEM((L, H * Dh), F32),
            pltpu.VMEM((n_seg, T, D), BF16),
            pltpu.VMEM((T, 128), F32),
            pltpu.VMEM((D // 2, F), U32),
            pltpu.VMEM((D // 2, F), U32),
            pltpu.VMEM((F // 2, D), U32),
            pltpu.VMEM((8, D), F32),
            pltpu.VMEM((8, D), F32),
            pltpu.VMEM((UNROLL, 4, 8, 128), F32),
            pltpu.SemaphoreType.DMA((NX,)),
            pltpu.SemaphoreType.DMA((6,)),
            pltpu.SemaphoreType.DMA((H,)),
            pltpu.SemaphoreType.DMA((H // 2,)),
            pltpu.SemaphoreType.DMA((H // 2,)),
            pltpu.SemaphoreType.DMA((3,)),
            pltpu.SemaphoreType.DMA((2,)),
        ],
        compiler_params=pltpu.CompilerParams(vmem_limit_bytes=120 * 1024 * 1024),
        name="rmt_mod_fused",
    )(
        A_x.reshape(n_seg, T, D),
        A_mem0.reshape(M, D),
        A_Wq.reshape(D // 2, 2, H, Dh),
        A_Wk.reshape(D // 2, 2, H, Dh),
        A_Wv.reshape(D // 2, 2, H, Dh),
        A_Wo.reshape(H * Dh, D),
        B_w_r,
        B_w_gate,
        B_w_up,
        B_w_down,
    )
    return out.reshape(B, S, D)
```

```python
import functools

import jax
import jax.numpy as jnp
from jax import lax
import jax.experimental.pallas as pl
import jax.experimental.pallas.tpu as pltpu

F32 = jnp.float32
BF16 = jnp.bfloat16
U32 = jnp.uint32

TOP_K = 2
LN_EPS = 1e-05
MASK_VALUE = -1000000000.0
LANES = 128
PRE = 8
UNROLL = 2

STREAM_PLAN = ((1, (2, 0, 0)), (1, (4, 0, 0)), (2, (4, 0, 0)), (4, (8, 0, 0)),
               (4, (8, 0, 0)), (8, (4, 6, 0)), (12, (0, 10, 16)))

ORDER_PLAIN = (2, 6, 16, 1)
ORDER_FFN = (1, 5, 24, 2)
FFN_AFTER_TILE = (0, 1, 2, 3, 6, 7)


def _rbf16(x):
    return x.astype(BF16).astype(F32)


def _dot(lhs, words):
    return jnp.dot(lhs, pltpu.bitcast(words, BF16), preferred_element_type=F32)


def _split_pair(w_ref, p):
    for r in range(0, w_ref.shape[1], 16):
        a = w_ref[2 * p, r:r + 16]
        b = w_ref[2 * p + 1, r:r + 16]
        w_ref[2 * p, r:r + 16] = (a & jnp.uint32(0xFFFF)) | (b << 16)
        w_ref[2 * p + 1, r:r + 16] = (a >> 16) | (b & jnp.uint32(0xFFFF0000))


def _start(copies):
    for cp in copies:
        cp.start()


def _wait(copies):
    for cp in copies:
        cp.wait()


def _kernel(x_hbm, mem0_hbm, wq_hbm, wk_hbm, wv_hbm, wo_hbm, wr_hbm, wg_hbm, wu_hbm, wd_hbm,
            out_hbm,
            xbuf, membuf, wrbuf, hall, wq, wk, wv, wo, qpre, kpre, obuf, outbuf, rbuf,
            wg, wu, wd, xsel, yacc, gu,
            sem_in, sem_qk, sem_v, sem_o, sem_ffn, sem_out):
    n_seg, T, D = xbuf.shape
    M = membuf.shape[0]
    H, _, Dh = wq.shape
    L = M + T
    scale = Dh ** (-0.5)
    n_pair = H // 2
    half_seg = n_seg // 2
    n_col = D // LANES
    n_ffn = wg.shape[1] // LANES

    wq32, wk32, wv32, wo32 = (r.bitcast(U32) for r in (wq_hbm, wk_hbm, wv_hbm, wo_hbm))

    def pair_copies(src, dst, p, sem):
        return [pltpu.make_async_copy(src.at[:, b, p, :], dst.at[2 * p + b], sem)
                for b in range(2)]

    def qk_copies(j):
        src, dst = ((wq32, wq), (wk32, wk))[j % 2]
        return pair_copies(src, dst, j // 2, sem_qk.at[j])

    def v_copies(p):
        return pair_copies(wv32, wv, p, sem_v.at[p])

    started = [0, 0, 0]
    cp_wo = []

    def start_weights(counts):
        for kind, copies in enumerate((qk_copies, v_copies)):
            for j in range(started[kind], started[kind] + counts[kind]):
                _start(copies(j))
        if counts[2]:
            rows = pl.ds(started[2] * Dh, counts[2] * Dh)
            cp_wo.append(pltpu.make_async_copy(wo32.at[rows], wo.at[rows], sem_o.at[len(cp_wo)]))
            cp_wo[-1].start()
        for kind in range(3):
            started[kind] += counts[kind]

    def x_copy(s0, s1, r0, r1, n):
        return pltpu.make_async_copy(x_hbm.at[s0:s1, r0:r1, :], xbuf.at[s0:s1, r0:r1, :],
                                     sem_in.at[n])

    cp_x_pre = [x_copy(0, half_seg, T - PRE, T, 0), x_copy(half_seg, n_seg, T - PRE, T, 1)]
    cp_x_early = [x_copy(0, 3, 0, T - PRE, 2), x_copy(half_seg + 1, half_seg + 2, 0, T - PRE, 3)]
    cp_x_late = [x_copy(3, half_seg + 1, 0, T - PRE, 4), x_copy(half_seg + 2, n_seg, 0, T - PRE, 5)]
    cp_small = [pltpu.make_async_copy(mem0_hbm, membuf, sem_in.at[6]),
                pltpu.make_async_copy(wr_hbm, wrbuf, sem_in.at[7])]
    cp_ffn = [pltpu.make_async_copy(src.bitcast(U32), dst, sem_ffn.at[n])
              for n, (src, dst) in enumerate(((wg_hbm, wg), (wu_hbm, wu), (wd_hbm, wd)))]

    def layernorm(s, r0, after=None):
        xs = xbuf[s, r0:r0 + 8, :].astype(F32)
        mean = jnp.mean(xs, axis=-1, keepdims=True)
        if after is not None:
            mean = jnp.maximum(mean, jnp.minimum(mean, jnp.where(after > 0, 1.0, 0.0)))
        cen = xs - mean
        var = jnp.mean(cen * cen, axis=-1, keepdims=True)
        den = _rbf16(jnp.sqrt(_rbf16(_rbf16(var) + LN_EPS)))
        xn = _rbf16(_rbf16(xs - _rbf16(mean)) / den)
        hall[s, M + r0:M + r0 + 8, :] = xn
        return xn

    def finish_segments(segs):
        lane = lax.broadcasted_iota(jnp.int32, (8, LANES), 1)
        w_r = wrbuf[...].astype(F32).reshape(1, D)
        r = None
        for s in segs:
            for r0 in range(0, T, 8):
                xn = layernorm(s, r0, r) if r0 < T - PRE else hall[s, M + r0:M + r0 + 8, :]
                r = _rbf16(jnp.sum(xn * w_r, axis=-1, keepdims=True))
                rbuf[r0:r0 + 8, :] = jnp.where(lane == s, r, rbuf[r0:r0 + 8, :])

    _start([cp_x_pre[0]] + cp_small + [cp_x_pre[1]])
    for c, cp in enumerate(cp_x_pre):
        cp.wait()
        start_weights((1, 0, 0))
        for s in range(c * half_seg, (c + 1) * half_seg):
            layernorm(s, T - PRE)
    _wait(cp_small)
    hall[0, :M, :] = membuf[...].astype(F32)
    rbuf[...] = jnp.full(rbuf.shape, -jnp.inf, F32)

    j0 = 0
    for g, (n_job, counts) in enumerate(STREAM_PLAN):
        for j in range(j0, j0 + n_job):
            _wait(qk_copies(j))
        start_weights(counts)
        if g == len(STREAM_PLAN) - 3:
            _start(cp_x_early)
        if g == len(STREAM_PLAN) - 1:
            _wait(cp_x_early)
        for j in range(j0, j0 + n_job):
            w_ref, pre = ((wq, qpre), (wk, kpre))[j % 2]
            _split_pair(w_ref, j // 2)
            for h in range(j // 2 * 2, j // 2 * 2 + 2):
                pre[h] = _dot(hall[:, L - PRE:, :].reshape(n_seg * PRE, D), w_ref[h])
        if g == len(STREAM_PLAN) - 1:
            finish_segments([0])
        j0 += n_job
    assert j0 == H and started == [H, n_pair, n_pair]
    for p in range(n_pair):
        _wait(v_copies(p))

    def route():
        seg_id = lax.broadcasted_iota(jnp.int32, (T, LANES), 1)
        tok = seg_id * T + lax.broadcasted_iota(jnp.int32, (T, LANES), 0)
        r_all = rbuf[...]
        key = jnp.where(r_all != r_all, -jnp.inf, r_all)
        live = seg_id < n_seg
        sub = lax.broadcasted_iota(jnp.int32, (8, D), 0)
        x_sel = jnp.zeros((8, D), F32)
        idx, gate = [], []
        for n in range(TOP_K):
            best = jnp.max(jnp.where(live, key, -jnp.inf), keepdims=True)
            first = jnp.min(jnp.where(live & (key == best), tok, n_seg * T), keepdims=True)
            live = live & (tok != first)
            i = first[0, 0]
            x_sel = jnp.where(sub == n, hall[i // T, pl.ds(M + i % T, 1), :], x_sel)
            idx.append(i)
            gate.append(jax.nn.sigmoid(best))
        xsel[...] = x_sel
        yacc[...] = jnp.zeros(yacc.shape, F32)
        return idx, gate

    def step(s, order, ffn_slice=None, first=False, last=False):
        lag_scores, lag_mix, h_split, c_split = order
        q0 = M if last else 0
        ri = q0 + lax.broadcasted_iota(jnp.int32, (L - q0, L), 0)
        ci = lax.broadcasted_iota(jnp.int32, (L - q0, L), 1)
        mask = (ri < M) | (ri >= ci)
        pre_rows = pl.ds(pl.multiple_of(s * PRE, PRE), PRE)
        qkv, prob, act = {}, {}, []

        def project(h):
            if first and h % 2 == 0:
                _split_pair(wv, h // 2)

            def over(d0, d1):
                d, w = slice(d0, d1), slice(d0 // 2, d1 // 2)
                return (_dot(hall[s, :L - PRE, d], wk[h, w]), _dot(hall[s, :L - PRE, d], wq[h, w]),
                        _dot(hall[s, :, d], wv[h, w]))

            if h == 0:
                k, q, v = (a + b for a, b in zip(over(0, D // 2), over(D // 2, D)))
            else:
                k, q, v = over(0, D)
            q = jnp.concatenate([q, qpre[h, pre_rows, :]], axis=0)
            k = jnp.concatenate([k, kpre[h, pre_rows, :]], axis=0)
            qkv[h] = (q[q0:], k.astype(BF16), v.astype(BF16))

        def scores(h):
            q, k, _ = qkv[h]
            sc = lax.dot_general(q, k, (((1,), (1,)), ((), ())), preferred_element_type=F32)
            sc = jnp.where(mask, sc * scale, MASK_VALUE)
            e = jnp.exp(sc - jnp.max(sc, axis=-1, keepdims=True))
            prob[h] = e / jnp.sum(e, axis=-1, keepdims=True)

        def mix(h):
            obuf[q0:, h * Dh:(h + 1) * Dh] = jnp.dot(prob.pop(h), qkv.pop(h)[2],
                                                     preferred_element_type=F32)

        def out_proj(h0, h1, c0, c1):
            return _dot(obuf[q0:, h0 * Dh:h1 * Dh],
                        wo[h0 * Dh // 2:h1 * Dh // 2, c0 * LANES:c1 * LANES])

        def ffn_piece(piece):
            t, slot, down = ffn_slice
            half = D // 2
            if piece == 0 and down:
                g = gu[slot, 0] + gu[slot, 1]
                act.append(g * jax.nn.sigmoid(g) * (gu[slot, 2] + gu[slot, 3]))
            if piece < 4:
                w_ref, k0 = (wg, wu)[piece // 2], piece % 2 * half
                cols = pl.ds(pl.multiple_of(jnp.minimum(t, n_ffn - 1) * LANES, LANES), LANES)
                gu[slot, piece] = _dot(xsel[:, k0:k0 + half], w_ref[k0 // 2:(k0 + half) // 2, cols])
            elif down:
                c0 = piece % 2 * half
                rows = pl.ds(pl.multiple_of((t - UNROLL) * (LANES // 2), LANES // 2), LANES // 2)
                yacc[:, c0:c0 + half] += _dot(act[0], wd[rows, c0:c0 + half])

        parts = []
        for i in range(H + n_col):
            if i < H:
                project(i)
            else:
                if i == H and first:
                    _wait(cp_wo)
                    _start(cp_x_late)
                parts.append(out_proj(0, h_split, i - H, i - H + 1))
            if ffn_slice is not None and i - H in FFN_AFTER_TILE:
                ffn_piece(FFN_AFTER_TILE.index(i - H))
            if 0 <= i - lag_scores < H:
                scores(i - lag_scores)
            if 0 <= i - lag_mix < H:
                mix(i - lag_mix)
        assert h_split + lag_mix <= H and not qkv
        hi = jnp.concatenate(parts[c_split:], axis=1) + out_proj(h_split, H, c_split, n_col)
        lo = jnp.concatenate(parts[:c_split], axis=1) + out_proj(h_split, H, 0, c_split)
        o = jnp.concatenate([lo, hi], axis=1)

        if not last:
            hall[s + 1, :M, :] = o[:M]
        outbuf[s] = (xbuf[s].astype(F32) + o[M - q0:] + hall[s, M:, :]).astype(BF16)

    s_ffn, s_last = half_seg, n_seg - 2
    assert s_last - s_ffn == n_ffn + UNROLL and (s_ffn - 2) % UNROLL == 0 and n_ffn % UNROLL == 0

    step(0, ORDER_PLAIN, first=True)
    finish_segments([1])
    step(1, ORDER_PLAIN)
    finish_segments([2, half_seg + 1])
    _wait(cp_x_late)
    _start(cp_ffn)

    def norm_steps(j, carry):
        for u in range(UNROLL):
            s = 2 + UNROLL * j + u
            step(s, ORDER_PLAIN)
            finish_segments([s + 1, s + half_seg])
        return carry

    lax.fori_loop(0, (s_ffn - 2) // UNROLL, norm_steps, 0)

    _wait(cp_ffn)
    idx, gate = route()
    for u in range(UNROLL):
        step(s_ffn + u, ORDER_FFN, ffn_slice=(u, u, False))

    def ffn_steps(j, carry):
        for u in range(UNROLL):
            step(s_ffn + UNROLL * j + u, ORDER_FFN, ffn_slice=(UNROLL * j + u, u, True))
        return carry

    lax.fori_loop(1, (s_last - s_ffn) // UNROLL, ffn_steps, 0)

    def write_out(s0, s1, sem):
        row = lax.broadcasted_iota(jnp.int32, (T, D), 0)
        for n, i in enumerate(idx):
            @pl.when((i >= s0 * T) & (i < s1 * T))
            def _():
                blk = outbuf[i // T].astype(F32)
                upd = yacc[n:n + 1, :] * gate[n]
                outbuf[i // T] = jnp.where(row == i % T, blk + upd, blk).astype(BF16)
        cp = pltpu.make_async_copy(outbuf.at[s0:s1], out_hbm.at[s0:s1], sem)
        cp.start()
        return cp

    cp_head = write_out(0, s_last, sem_out.at[0])
    for s in range(s_last, n_seg):
        step(s, ORDER_PLAIN, last=s == n_seg - 1)
    _wait([cp_head, write_out(s_last, n_seg, sem_out.at[1])])


@functools.partial(jax.jit, static_argnames=("A_seg_len",))
def pallas_parallel_sum__memory_aug_recurrent_mem_tr__moe_arch_mod__prompt_kernel(
    A_x: jax.Array,
    A_mem0: jax.Array,
    A_Wq: jax.Array,
    A_Wk: jax.Array,
    A_Wv: jax.Array,
    A_Wo: jax.Array,
    A_seg_len: int,
    B_x: jax.Array,
    B_w_r: jax.Array,
    B_w_gate: jax.Array,
    B_w_up: jax.Array,
    B_w_down: jax.Array,
):
    del B_x
    B, S, D = A_x.shape
    _, H, Dh = A_Wq.shape
    M = A_mem0.shape[1]
    T = int(A_seg_len)
    F = B_w_gate.shape[1]
    L = M + T
    n_seg = S // T
    assert B == 1 and S % T == 0 and T % 16 == 0 and M % 8 == 0 and Dh == LANES and H % 2 == 0
    assert n_seg <= LANES

    any_spec = pl.BlockSpec(memory_space=pl.ANY)
    out = pl.pallas_call(
        _kernel,
        out_shape=jax.ShapeDtypeStruct((n_seg, T, D), A_x.dtype),
        in_specs=[any_spec] * 10,
        out_specs=any_spec,
        scratch_shapes=[
            pltpu.VMEM((n_seg, T, D), BF16),
            pltpu.VMEM((M, D), BF16),
            pltpu.VMEM((D,), BF16),
            pltpu.VMEM((n_seg, L, D), F32),
            pltpu.VMEM((H, D // 2, Dh), U32),
            pltpu.VMEM((H, D // 2, Dh), U32),
            pltpu.VMEM((H, D // 2, Dh), U32),
            pltpu.VMEM((H * Dh // 2, D), U32),
            pltpu.VMEM((H, n_seg * PRE, Dh), F32),
            pltpu.VMEM((H, n_seg * PRE, Dh), F32),
            pltpu.VMEM((L, H * Dh), F32),
            pltpu.VMEM((n_seg, T, D), BF16),
            pltpu.VMEM((T, LANES), F32),
            pltpu.VMEM((D // 2, F), U32),
            pltpu.VMEM((D // 2, F), U32),
            pltpu.VMEM((F // 2, D), U32),
            pltpu.VMEM((8, D), F32),
            pltpu.VMEM((8, D), F32),
            pltpu.VMEM((UNROLL, 4, 8, LANES), F32),
            pltpu.SemaphoreType.DMA((8,)),
            pltpu.SemaphoreType.DMA((H,)),
            pltpu.SemaphoreType.DMA((H // 2,)),
            pltpu.SemaphoreType.DMA((len(STREAM_PLAN),)),
            pltpu.SemaphoreType.DMA((3,)),
            pltpu.SemaphoreType.DMA((2,)),
        ],
        compiler_params=pltpu.CompilerParams(vmem_limit_bytes=120 * 1024 * 1024),
        name="rmt_mod_fused",
    )(
        A_x.reshape(n_seg, T, D),
        A_mem0.reshape(M, D),
        A_Wq.reshape(D // 2, 2, H, Dh),
        A_Wk.reshape(D // 2, 2, H, Dh),
        A_Wv.reshape(D // 2, 2, H, Dh),
        A_Wo.reshape(H * Dh, D),
        B_w_r,
        B_w_gate,
        B_w_up,
        B_w_down,
    )
    return out.reshape(B, S, D)
```

```python
import functools

import jax
import jax.numpy as jnp
from jax import lax
import jax.experimental.pallas as pl
import jax.experimental.pallas.tpu as pltpu

F32 = jnp.float32
BF16 = jnp.bfloat16
U32 = jnp.uint32

TOP_K = 2
LN_EPS = 1e-05
MASK_VALUE = -1000000000.0
LANES = 128
PRE = 8
V_EARLY = (0, 1, 15)
UNROLL = 2

STREAM_PLAN = ((1, 2, 0), (1, 3, 0), (2, 5, 0), (3, 9, 0), (5, 10, 0), (9, 4, 6), (14, 0, 7))

ORDER_PLAIN = (2, 5, 20, 2)
ORDER_FFN = (2, 4, 24, 2)
FFN_AFTER_TILE = (0, 1, 2, 3, 6, 7)


def _rbf16(x):
    return x.astype(BF16).astype(F32)


def _dot(lhs, words):
    return jnp.dot(lhs, pltpu.bitcast(words, BF16), preferred_element_type=F32)


def _split_pair(w_ref, p):
    for r in range(0, w_ref.shape[1], 16):
        a = w_ref[2 * p, r:r + 16]
        b = w_ref[2 * p + 1, r:r + 16]
        w_ref[2 * p, r:r + 16] = (a & jnp.uint32(0xFFFF)) | (b << 16)
        w_ref[2 * p + 1, r:r + 16] = (a >> 16) | (b & jnp.uint32(0xFFFF0000))


def _combine(a, b, op):
    halves = [op(pltpu.bitcast(half(a), F32), pltpu.bitcast(half(b), F32))
              for half in (lambda w: w << 16, lambda w: w & jnp.uint32(0xFFFF0000))]
    return pltpu.bitcast(pltpu.pack_elementwise(halves, packed_dtype=BF16), U32)


def _start(copies):
    for cp in copies:
        cp.start()


def _wait(copies):
    for cp in copies:
        cp.wait()


def _kernel(x_hbm, mem0_hbm, wq_hbm, wk_hbm, wv_hbm, wo_hbm, wr_hbm, wg_hbm, wu_hbm, wd_hbm,
            out_hbm,
            xbuf, membuf, wrbuf, hall, wq, wk, wv, wo, qpre, kpre, vpre, xsum, obuf, outbuf, rbuf,
            wg, wu, wd, xsel, yacc, gu,
            sem_in, sem_w, sem_ffn, sem_out):
    n_seg, T, D = xbuf.shape
    M = membuf.shape[0]
    H, _, Dh = wq.shape
    L = M + T
    scale = Dh ** (-0.5)
    n_pair = H // 2
    half_seg = n_seg // 2
    n_col = D // LANES
    n_ffn = wg.shape[1] // LANES

    wq32, wk32, wv32, wo32 = (r.bitcast(U32) for r in (wq_hbm, wk_hbm, wv_hbm, wo_hbm))

    jobs = []
    for p in range(n_pair):
        jobs += [(p, wq32, wq, qpre, 2 * p), (p, wk32, wk, kpre, 2 * p)]
        if p in V_EARLY:
            jobs.append((p, wv32, wv, vpre, 2 * V_EARLY.index(p)))
    n_early = len(jobs)
    jobs += [(p, wv32, wv) for p in range(n_pair) if p not in V_EARLY]

    def job_copies(j):
        p, src, dst = jobs[j][:3]
        return [pltpu.make_async_copy(src.at[:, b, p, :], dst.at[2 * p + b], sem_w.at[j])
                for b in range(2)]

    def x_copy(s0, s1, r0, r1, n):
        return pltpu.make_async_copy(x_hbm.at[s0:s1, r0:r1, :], xbuf.at[s0:s1, r0:r1, :],
                                     sem_in.at[n])

    cp_x_pre = [x_copy(0, half_seg, T - PRE, T, 0), x_copy(half_seg, n_seg, T - PRE, T, 1)]
    cp_x_early = [x_copy(0, 3, 0, T - PRE, 2), x_copy(half_seg + 1, half_seg + 2, 0, T - PRE, 3)]
    cp_x_late = [x_copy(3, half_seg + 1, 0, T - PRE, 4), x_copy(half_seg + 2, n_seg, 0, T - PRE, 5)]
    cp_small = [pltpu.make_async_copy(mem0_hbm, membuf, sem_in.at[6]),
                pltpu.make_async_copy(wr_hbm, wrbuf, sem_in.at[7])]
    cp_wo = pltpu.make_async_copy(wo32, wo, sem_in.at[8])
    cp_ffn = [pltpu.make_async_copy(src.bitcast(U32), dst, sem_ffn.at[n])
              for n, (src, dst) in enumerate(((wg_hbm, wg), (wu_hbm, wu), (wd_hbm, wd)))]

    def layernorm(s, r0, after=None):
        xs = xbuf[s, r0:r0 + 8, :].astype(F32)
        mean = jnp.mean(xs, axis=-1, keepdims=True)
        if after is not None:
            mean = jnp.maximum(mean, jnp.minimum(mean, jnp.where(after > 0, 1.0, 0.0)))
        cen = xs - mean
        var = jnp.mean(cen * cen, axis=-1, keepdims=True)
        den = _rbf16(jnp.sqrt(_rbf16(_rbf16(var) + LN_EPS)))
        xn = _rbf16(_rbf16(xs - _rbf16(mean)) / den)
        hall[s, M + r0:M + r0 + 8, :] = xn
        return xn

    def finish_segments(segs):
        lane = lax.broadcasted_iota(jnp.int32, (8, LANES), 1)
        w_r = wrbuf[...].astype(F32).reshape(1, D)
        r = None
        for s in segs:
            for r0 in range(0, T, 8):
                xn = layernorm(s, r0, r) if r0 < T - PRE else hall[s, M + r0:M + r0 + 8, :]
                r = _rbf16(jnp.sum(xn * w_r, axis=-1, keepdims=True))
                rbuf[r0:r0 + 8, :] = jnp.where(lane == s, r, rbuf[r0:r0 + 8, :])

    _start([cp_x_pre[0]] + cp_small + [cp_x_pre[1]])
    for c, cp in enumerate(cp_x_pre):
        cp.wait()
        _start(job_copies(c))
        for s in range(c * half_seg, (c + 1) * half_seg):
            layernorm(s, T - PRE)
    _wait(cp_small)
    hall[0, :M, :] = membuf[...].astype(F32)
    rbuf[...] = jnp.full(rbuf.shape, -jnp.inf, F32)

    n_half = half_seg * PRE

    def x_sums():
        for s in range(half_seg):
            top, bottom = hall[s, L - PRE:, :], hall[half_seg + s, L - PRE:, :]
            x11, x12 = top[:, :D // 2], top[:, D // 2:]
            x21, x22 = bottom[:, :D // 2], bottom[:, D // 2:]
            for n, v in enumerate((x11 + x22, x21 + x22, x11 + x12, x21 - x11, x12 - x22)):
                xsum[n, s * PRE:(s + 1) * PRE] = v

    def project_early(j):
        p, _, w_ref, pre, h = jobs[j]

        def x_diag(i):
            return hall[i * half_seg:(i + 1) * half_seg, L - PRE:,
                        i * D // 2:(i + 1) * D // 2].reshape(n_half, D // 2)

        def w(i, c):
            return w_ref[2 * p + c, i * D // 4:(i + 1) * D // 4]

        _split_pair(w_ref, p)
        m3 = _dot(x_diag(0), _combine(w(0, 1), w(1, 1), jnp.subtract))
        m4 = _dot(x_diag(1), _combine(w(1, 0), w(0, 0), jnp.subtract))
        m5 = _dot(xsum[2], w(1, 1))
        pre[h + 1, :n_half] = m3 + m5
        m2 = _dot(xsum[1], w(0, 0))
        pre[h, n_half:] = m2 + m4
        m1 = _dot(xsum[0], _combine(w(0, 0), w(1, 1), jnp.add))
        pre[h, :n_half] = (m4 - m5) + m1 + _dot(xsum[4], _combine(w(1, 0), w(1, 1), jnp.add))
        pre[h + 1, n_half:] = (m3 - m2) + m1 + _dot(xsum[3], _combine(w(0, 0), w(0, 1), jnp.add))

    done, early, late = 0, len(cp_x_pre), n_early
    for g, (n_run, n_start, n_late) in enumerate(STREAM_PLAN):
        for j in range(done, done + n_run):
            _wait(job_copies(j))
        for j in [*range(early, early + n_start), *range(late, late + n_late)]:
            _start(job_copies(j))
        if g == len(STREAM_PLAN) - 3:
            _start(cp_x_early)
        if g == len(STREAM_PLAN) - 1:
            cp_wo.start()
            _wait(cp_x_early)
        if g == 0:
            x_sums()
        for j in range(done, done + n_run):
            project_early(j)
        if g == len(STREAM_PLAN) - 1:
            finish_segments([0])
        done, early, late = done + n_run, early + n_start, late + n_late
    assert done == early == n_early and late == len(jobs)
    for j in range(n_early, len(jobs)):
        _wait(job_copies(j))

    def route():
        seg_id = lax.broadcasted_iota(jnp.int32, (T, LANES), 1)
        tok = seg_id * T + lax.broadcasted_iota(jnp.int32, (T, LANES), 0)
        r_all = rbuf[...]
        key = jnp.where(r_all != r_all, -jnp.inf, r_all)
        live = seg_id < n_seg
        sub = lax.broadcasted_iota(jnp.int32, (8, D), 0)
        x_sel = jnp.zeros((8, D), F32)
        idx, gate = [], []
        for n in range(TOP_K):
            best = jnp.max(jnp.where(live, key, -jnp.inf), keepdims=True)
            first = jnp.min(jnp.where(live & (key == best), tok, n_seg * T), keepdims=True)
            live = live & (tok != first)
            i = first[0, 0]
            x_sel = jnp.where(sub == n, hall[i // T, pl.ds(M + i % T, 1), :], x_sel)
            idx.append(i)
            gate.append(jax.nn.sigmoid(best))
        xsel[...] = x_sel
        yacc[...] = jnp.zeros(yacc.shape, F32)
        return idx, gate

    def step(s, order, ffn_slice=None, first=False, last=False):
        lag_scores, lag_mix, h_split, c_split = order
        q0 = M if last else 0
        ri = q0 + lax.broadcasted_iota(jnp.int32, (L - q0, L), 0)
        ci = lax.broadcasted_iota(jnp.int32, (L - q0, L), 1)
        mask = (ri < M) | (ri >= ci)
        pre_rows = pl.ds(pl.multiple_of(s * PRE, PRE), PRE)
        qkv, prob, act = {}, {}, []

        def project(h):
            p = h // 2
            if first and h % 2 == 0 and p not in V_EARLY:
                _split_pair(wv, p)
            rows = (L - PRE, L - PRE, L - PRE if p in V_EARLY else L)

            def over(d0, d1):
                return [_dot(hall[s, :n, d0:d1], w_ref[h, d0 // 2:d1 // 2])
                        for w_ref, n in zip((wk, wq, wv), rows)]

            if h == 0:
                k, q, v = [a + b for a, b in zip(over(0, D // 2), over(D // 2, D))]
            else:
                k, q, v = over(0, D)
            q = jnp.concatenate([q, qpre[h, pre_rows, :]], axis=0)
            k = jnp.concatenate([k, kpre[h, pre_rows, :]], axis=0)
            if p in V_EARLY:
                v = jnp.concatenate([v, vpre[2 * V_EARLY.index(p) + h % 2, pre_rows, :]], axis=0)
            qkv[h] = (q[q0:], k.astype(BF16), v.astype(BF16))

        def scores(h):
            q, k, _ = qkv[h]
            sc = lax.dot_general(q, k, (((1,), (1,)), ((), ())), preferred_element_type=F32)
            sc = jnp.where(mask, sc * scale, MASK_VALUE)
            e = jnp.exp(sc - jnp.max(sc, axis=-1, keepdims=True))
            prob[h] = e / jnp.sum(e, axis=-1, keepdims=True)

        def mix(h):
            obuf[q0:, h * Dh:(h + 1) * Dh] = jnp.dot(prob.pop(h), qkv.pop(h)[2],
                                                     preferred_element_type=F32)

        def out_proj(h0, h1, c0, c1):
            return _dot(obuf[q0:, h0 * Dh:h1 * Dh],
                        wo[h0 * Dh // 2:h1 * Dh // 2, c0 * LANES:c1 * LANES])

        def ffn_piece(piece):
            t, slot, down = ffn_slice
            half = D // 2
            if piece == 0 and down:
                g = gu[slot, 0] + gu[slot, 1]
                act.append(g * jax.nn.sigmoid(g) * (gu[slot, 2] + gu[slot, 3]))
            if piece < 4:
                w_ref, k0 = (wg, wu)[piece // 2], piece % 2 * half
                cols = pl.ds(pl.multiple_of(jnp.minimum(t, n_ffn - 1) * LANES, LANES), LANES)
                gu[slot, piece] = _dot(xsel[:, k0:k0 + half], w_ref[k0 // 2:(k0 + half) // 2, cols])
            elif down:
                c0 = piece % 2 * half
                rows = pl.ds(pl.multiple_of((t - UNROLL) * (LANES // 2), LANES // 2), LANES // 2)
                yacc[:, c0:c0 + half] += _dot(act[0], wd[rows, c0:c0 + half])

        parts = []
        for i in range(H + n_col):
            if i < H:
                project(i)
            else:
                if i == H and first:
                    cp_wo.wait()
                    _start(cp_x_late)
                parts.append(out_proj(0, h_split, i - H, i - H + 1))
            if ffn_slice is not None and i - H in FFN_AFTER_TILE:
                ffn_piece(FFN_AFTER_TILE.index(i - H))
            if 0 <= i - lag_scores < H:
                scores(i - lag_scores)
            if 0 <= i - lag_mix < H:
                mix(i - lag_mix)
        assert h_split + lag_mix <= H and not qkv
        hi = jnp.concatenate(parts[c_split:], axis=1) + out_proj(h_split, H, c_split, n_col)
        lo = jnp.concatenate(parts[:c_split], axis=1) + out_proj(h_split, H, 0, c_split)
        o = jnp.concatenate([lo, hi], axis=1)

        if not last:
            hall[s + 1, :M, :] = o[:M]
        outbuf[s] = (xbuf[s].astype(F32) + o[M - q0:] + hall[s, M:, :]).astype(BF16)

    s_ffn, s_last = half_seg, n_seg - 2
    assert s_last - s_ffn == n_ffn + UNROLL and (s_ffn - 2) % UNROLL == 0 and n_ffn % UNROLL == 0

    step(0, ORDER_PLAIN, first=True)
    finish_segments([1])
    step(1, ORDER_PLAIN)
    finish_segments([2, half_seg + 1])
    _wait(cp_x_late)
    _start(cp_ffn)

    def norm_steps(j, carry):
        for u in range(UNROLL):
            s = 2 + UNROLL * j + u
            step(s, ORDER_PLAIN)
            finish_segments([s + 1, s + half_seg])
        return carry

    lax.fori_loop(0, (s_ffn - 2) // UNROLL, norm_steps, 0)

    _wait(cp_ffn)
    idx, gate = route()
    for u in range(UNROLL):
        step(s_ffn + u, ORDER_FFN, ffn_slice=(u, u, False))

    def ffn_steps(j, carry):
        for u in range(UNROLL):
            step(s_ffn + UNROLL * j + u, ORDER_FFN, ffn_slice=(UNROLL * j + u, u, True))
        return carry

    lax.fori_loop(1, (s_last - s_ffn) // UNROLL, ffn_steps, 0)

    def write_out(s0, s1, sem):
        row = lax.broadcasted_iota(jnp.int32, (T, D), 0)
        for n, i in enumerate(idx):
            @pl.when((i >= s0 * T) & (i < s1 * T))
            def _():
                blk = outbuf[i // T].astype(F32)
                upd = yacc[n:n + 1, :] * gate[n]
                outbuf[i // T] = jnp.where(row == i % T, blk + upd, blk).astype(BF16)
        cp = pltpu.make_async_copy(outbuf.at[s0:s1], out_hbm.at[s0:s1], sem)
        cp.start()
        return cp

    cp_head = write_out(0, s_last, sem_out.at[0])
    for s in range(s_last, n_seg):
        step(s, ORDER_PLAIN, last=s == n_seg - 1)
    _wait([cp_head, write_out(s_last, n_seg, sem_out.at[1])])


@functools.partial(jax.jit, static_argnames=("A_seg_len",))
def pallas_parallel_sum__memory_aug_recurrent_mem_tr__moe_arch_mod__prompt_kernel(
    A_x: jax.Array,
    A_mem0: jax.Array,
    A_Wq: jax.Array,
    A_Wk: jax.Array,
    A_Wv: jax.Array,
    A_Wo: jax.Array,
    A_seg_len: int,
    B_x: jax.Array,
    B_w_r: jax.Array,
    B_w_gate: jax.Array,
    B_w_up: jax.Array,
    B_w_down: jax.Array,
):
    del B_x
    B, S, D = A_x.shape
    _, H, Dh = A_Wq.shape
    M = A_mem0.shape[1]
    T = int(A_seg_len)
    F = B_w_gate.shape[1]
    L = M + T
    n_seg = S // T
    assert B == 1 and S % T == 0 and T % 16 == 0 and M % 8 == 0 and Dh == LANES and H % 2 == 0
    assert n_seg <= LANES

    any_spec = pl.BlockSpec(memory_space=pl.ANY)
    out = pl.pallas_call(
        _kernel,
        out_shape=jax.ShapeDtypeStruct((n_seg, T, D), A_x.dtype),
        in_specs=[any_spec] * 10,
        out_specs=any_spec,
        scratch_shapes=[
            pltpu.VMEM((n_seg, T, D), BF16),
            pltpu.VMEM((M, D), BF16),
            pltpu.VMEM((D,), BF16),
            pltpu.VMEM((n_seg, L, D), F32),
            pltpu.VMEM((H, D // 2, Dh), U32),
            pltpu.VMEM((H, D // 2, Dh), U32),
            pltpu.VMEM((H, D // 2, Dh), U32),
            pltpu.VMEM((H * Dh // 2, D), U32),
            pltpu.VMEM((H, n_seg * PRE, Dh), F32),
            pltpu.VMEM((H, n_seg * PRE, Dh), F32),
            pltpu.VMEM((2 * len(V_EARLY), n_seg * PRE, Dh), F32),
            pltpu.VMEM((5, n_seg * PRE // 2, D // 2), F32),
            pltpu.VMEM((L, H * Dh), F32),
            pltpu.VMEM((n_seg, T, D), BF16),
            pltpu.VMEM((T, LANES), F32),
            pltpu.VMEM((D // 2, F), U32),
            pltpu.VMEM((D // 2, F), U32),
            pltpu.VMEM((F // 2, D), U32),
            pltpu.VMEM((8, D), F32),
            pltpu.VMEM((8, D), F32),
            pltpu.VMEM((UNROLL, 4, 8, LANES), F32),
            pltpu.SemaphoreType.DMA((9,)),
            pltpu.SemaphoreType.DMA((3 * H // 2,)),
            pltpu.SemaphoreType.DMA((3,)),
            pltpu.SemaphoreType.DMA((2,)),
        ],
        compiler_params=pltpu.CompilerParams(vmem_limit_bytes=120 * 1024 * 1024),
        name="rmt_mod_fused",
    )(
        A_x.reshape(n_seg, T, D),
        A_mem0.reshape(M, D),
        A_Wq.reshape(D // 2, 2, H, Dh),
        A_Wk.reshape(D // 2, 2, H, Dh),
        A_Wv.reshape(D // 2, 2, H, Dh),
        A_Wo.reshape(H * Dh, D),
        B_w_r,
        B_w_gate,
        B_w_up,
        B_w_down,
    )
    return out.reshape(B, S, D)
```

```python
import functools

import jax
import jax.numpy as jnp
import numpy as np
from jax import lax
import jax.experimental.pallas as pl
import jax.experimental.pallas.tpu as pltpu

F32 = jnp.float32
BF16 = jnp.bfloat16
U32 = jnp.uint32
LOW_HALF = np.uint32(0x0000FFFF)
HIGH_HALF = np.uint32(0xFFFF0000)

TOP_K = 2
LN_EPS = 1e-05
MASK_VALUE = -1000000000.0
LANES = 128
PRE = 8
V_EARLY = (0, 1, 15)
UNROLL = 2

STREAM_PLAN = ((1, 2, 0), (1, 3, 0), (2, 5, 0), (3, 9, 0), (5, 10, 0), (9, 4, 6), (14, 0, 7))

ORDER_PLAIN = (2, 5, 20, 2)
ORDER_FFN = (2, 4, 24, 2)
FFN_AFTER_TILE = (0, 1, 2, 3, 6, 7)


def _rbf16(x):
    return x.astype(BF16).astype(F32)


def _dot(lhs, words):
    return jnp.dot(lhs, pltpu.bitcast(words, BF16), preferred_element_type=F32)


def _split_pair(w_ref, p):
    for r in range(0, w_ref.shape[1], 16):
        a = w_ref[2 * p, r:r + 16]
        b = w_ref[2 * p + 1, r:r + 16]
        w_ref[2 * p, r:r + 16] = (a & LOW_HALF) | (b << 16)
        w_ref[2 * p + 1, r:r + 16] = (a >> 16) | (b & HIGH_HALF)


def _combine(a, b, op):
    low, high = (
        pltpu.bitcast(_rbf16(op(pltpu.bitcast(half(a), F32), pltpu.bitcast(half(b), F32))), U32)
        for half in (lambda w: w << 16, lambda w: w & HIGH_HALF))
    return (low >> 16) | high


def _start(copies):
    for cp in copies:
        cp.start()


def _wait(copies):
    for cp in copies:
        cp.wait()


def _kernel(x_hbm, mem0_hbm, wq_hbm, wk_hbm, wv_hbm, wo_hbm, wr_hbm, wg_hbm, wu_hbm, wd_hbm,
            out_hbm,
            xbuf, membuf, wrbuf, hall, wq, wk, wv, wo, qpre, kpre, vpre, xsum, obuf, outbuf, rbuf,
            wg, wu, wd, xsel, yacc, gu,
            sem_in, sem_w, sem_ffn, sem_out):
    n_seg, T, D = xbuf.shape
    M = membuf.shape[0]
    H, _, Dh = wq.shape
    L = M + T
    scale = Dh ** (-0.5)
    n_pair = H // 2
    half_seg = n_seg // 2
    n_col = D // LANES
    n_ffn = wg.shape[1] // LANES

    wq32, wk32, wv32, wo32 = (r.bitcast(U32) for r in (wq_hbm, wk_hbm, wv_hbm, wo_hbm))

    jobs = []
    for p in range(n_pair):
        jobs += [(p, wq32, wq, qpre, 2 * p), (p, wk32, wk, kpre, 2 * p)]
        if p in V_EARLY:
            jobs.append((p, wv32, wv, vpre, 2 * V_EARLY.index(p)))
    n_early = len(jobs)
    jobs += [(p, wv32, wv) for p in range(n_pair) if p not in V_EARLY]

    def job_copies(j):
        p, src, dst = jobs[j][:3]
        return [pltpu.make_async_copy(src.at[:, b, p, :], dst.at[2 * p + b], sem_w.at[j])
                for b in range(2)]

    def x_copy(s0, s1, r0, r1, n):
        return pltpu.make_async_copy(x_hbm.at[s0:s1, r0:r1, :], xbuf.at[s0:s1, r0:r1, :],
                                     sem_in.at[n])

    cp_x_pre = [x_copy(0, half_seg, T - PRE, T, 0), x_copy(half_seg, n_seg, T - PRE, T, 1)]
    cp_x_early = [x_copy(0, 3, 0, T - PRE, 2), x_copy(half_seg + 1, half_seg + 2, 0, T - PRE, 3)]
    cp_x_late = [x_copy(3, half_seg + 1, 0, T - PRE, 4), x_copy(half_seg + 2, n_seg, 0, T - PRE, 5)]
    cp_small = [pltpu.make_async_copy(mem0_hbm, membuf, sem_in.at[6]),
                pltpu.make_async_copy(wr_hbm, wrbuf, sem_in.at[7])]
    cp_wo = pltpu.make_async_copy(wo32, wo, sem_in.at[8])
    cp_ffn = [pltpu.make_async_copy(src.bitcast(U32), dst, sem_ffn.at[n])
              for n, (src, dst) in enumerate(((wg_hbm, wg), (wu_hbm, wu), (wd_hbm, wd)))]

    def layernorm(s, r0, after=None):
        xs = xbuf[s, r0:r0 + 8, :].astype(F32)
        mean = jnp.mean(xs, axis=-1, keepdims=True)
        if after is not None:
            mean = jnp.maximum(mean, jnp.minimum(mean, jnp.where(after > 0, 1.0, 0.0)))
        cen = xs - mean
        var = jnp.mean(cen * cen, axis=-1, keepdims=True)
        den = _rbf16(jnp.sqrt(_rbf16(_rbf16(var) + LN_EPS)))
        xn = _rbf16(_rbf16(xs - _rbf16(mean)) / den)
        hall[s, M + r0:M + r0 + 8, :] = xn
        return xn

    def finish_segments(segs):
        lane = lax.broadcasted_iota(jnp.int32, (8, LANES), 1)
        w_r = wrbuf[...].astype(F32).reshape(1, D)
        r = None
        for s in segs:
            for r0 in range(0, T, 8):
                xn = layernorm(s, r0, r) if r0 < T - PRE else hall[s, M + r0:M + r0 + 8, :]
                r = _rbf16(jnp.sum(xn * w_r, axis=-1, keepdims=True))
                rbuf[r0:r0 + 8, :] = jnp.where(lane == s, r, rbuf[r0:r0 + 8, :])

    _start([cp_x_pre[0]] + cp_small + [cp_x_pre[1]])
    for c, cp in enumerate(cp_x_pre):
        cp.wait()
        _start(job_copies(c))
        for s in range(c * half_seg, (c + 1) * half_seg):
            layernorm(s, T - PRE)
    _wait(cp_small)
    hall[0, :M, :] = membuf[...].astype(F32)
    rbuf[...] = jnp.full(rbuf.shape, -jnp.inf, F32)

    n_half = half_seg * PRE

    def x_sums():
        for s in range(half_seg):
            top, bottom = hall[s, L - PRE:, :], hall[half_seg + s, L - PRE:, :]
            x11, x12 = top[:, :D // 2], top[:, D // 2:]
            x21, x22 = bottom[:, :D // 2], bottom[:, D // 2:]
            for n, v in enumerate((x11 + x22, x21 + x22, x11 + x12, x21 - x11, x12 - x22)):
                xsum[n, s * PRE:(s + 1) * PRE] = v

    def project_early(j):
        p, _, w_ref, pre, h = jobs[j]

        def x_diag(i):
            return hall[i * half_seg:(i + 1) * half_seg, L - PRE:,
                        i * D // 2:(i + 1) * D // 2].reshape(n_half, D // 2)

        def w(i, c):
            return w_ref[2 * p + c, i * D // 4:(i + 1) * D // 4]

        _split_pair(w_ref, p)
        m3 = _dot(x_diag(0), _combine(w(0, 1), w(1, 1), jnp.subtract))
        m4 = _dot(x_diag(1), _combine(w(1, 0), w(0, 0), jnp.subtract))
        m5 = _dot(xsum[2], w(1, 1))
        pre[h + 1, :n_half] = m3 + m5
        m2 = _dot(xsum[1], w(0, 0))
        pre[h, n_half:] = m2 + m4
        m1 = _dot(xsum[0], _combine(w(0, 0), w(1, 1), jnp.add))
        pre[h, :n_half] = (m4 - m5) + m1 + _dot(xsum[4], _combine(w(1, 0), w(1, 1), jnp.add))
        pre[h + 1, n_half:] = (m3 - m2) + m1 + _dot(xsum[3], _combine(w(0, 0), w(0, 1), jnp.add))

    done, early, late = 0, len(cp_x_pre), n_early
    for g, (n_run, n_start, n_late) in enumerate(STREAM_PLAN):
        for j in range(done, done + n_run):
            _wait(job_copies(j))
        for j in [*range(early, early + n_start), *range(late, late + n_late)]:
            _start(job_copies(j))
        if g == len(STREAM_PLAN) - 3:
            _start(cp_x_early)
        if g == len(STREAM_PLAN) - 1:
            cp_wo.start()
            _wait(cp_x_early)
        if g == 0:
            x_sums()
        for j in range(done, done + n_run):
            project_early(j)
        if g == len(STREAM_PLAN) - 1:
            finish_segments([0])
        done, early, late = done + n_run, early + n_start, late + n_late
    assert done == early == n_early and late == len(jobs)
    for j in range(n_early, len(jobs)):
        _wait(job_copies(j))

    def route():
        seg_id = lax.broadcasted_iota(jnp.int32, (T, LANES), 1)
        tok = seg_id * T + lax.broadcasted_iota(jnp.int32, (T, LANES), 0)
        r_all = rbuf[...]
        key = jnp.where(r_all != r_all, -jnp.inf, r_all)
        live = seg_id < n_seg
        sub = lax.broadcasted_iota(jnp.int32, (8, D), 0)
        x_sel = jnp.zeros((8, D), F32)
        idx, gate = [], []
        for n in range(TOP_K):
            best = jnp.max(jnp.where(live, key, -jnp.inf), keepdims=True)
            first = jnp.min(jnp.where(live & (key == best), tok, n_seg * T), keepdims=True)
            live = live & (tok != first)
            i = first[0, 0]
            x_sel = jnp.where(sub == n, hall[i // T, pl.ds(M + i % T, 1), :], x_sel)
            idx.append(i)
            gate.append(jax.nn.sigmoid(best))
        xsel[...] = x_sel
        yacc[...] = jnp.zeros(yacc.shape, F32)
        return idx, gate

    def step(s, order, ffn_slice=None, first=False, last=False):
        lag_scores, lag_mix, h_split, c_split = order
        q0 = M if last else 0
        ri = q0 + lax.broadcasted_iota(jnp.int32, (L - q0, L), 0)
        ci = lax.broadcasted_iota(jnp.int32, (L - q0, L), 1)
        mask = (ri < M) | (ri >= ci)
        pre_rows = pl.ds(pl.multiple_of(s * PRE, PRE), PRE)
        qkv, prob, act = {}, {}, []

        def project(h):
            p = h // 2
            if first and h % 2 == 0 and p not in V_EARLY:
                _split_pair(wv, p)
            rows = (L - PRE, L - PRE, L - PRE if p in V_EARLY else L)

            def over(d0, d1):
                return [_dot(hall[s, :n, d0:d1], w_ref[h, d0 // 2:d1 // 2])
                        for w_ref, n in zip((wk, wq, wv), rows)]

            if h == 0:
                k, q, v = [a + b for a, b in zip(over(0, D // 2), over(D // 2, D))]
            else:
                k, q, v = over(0, D)
            q = jnp.concatenate([q, qpre[h, pre_rows, :]], axis=0)
            k = jnp.concatenate([k, kpre[h, pre_rows, :]], axis=0)
            if p in V_EARLY:
                v = jnp.concatenate([v, vpre[2 * V_EARLY.index(p) + h % 2, pre_rows, :]], axis=0)
            qkv[h] = (q[q0:], k.astype(BF16), v.astype(BF16))

        def scores(h):
            q, k, _ = qkv[h]
            sc = lax.dot_general(q, k, (((1,), (1,)), ((), ())), preferred_element_type=F32)
            sc = jnp.where(mask, sc * scale, MASK_VALUE)
            e = jnp.exp(sc - jnp.max(sc, axis=-1, keepdims=True))
            prob[h] = e / jnp.sum(e, axis=-1, keepdims=True)

        def mix(h):
            obuf[q0:, h * Dh:(h + 1) * Dh] = jnp.dot(prob.pop(h), qkv.pop(h)[2],
                                                     preferred_element_type=F32)

        def out_proj(h0, h1, c0, c1):
            return _dot(obuf[q0:, h0 * Dh:h1 * Dh],
                        wo[h0 * Dh // 2:h1 * Dh // 2, c0 * LANES:c1 * LANES])

        def ffn_piece(piece):
            t, slot, down = ffn_slice
            half = D // 2
            if piece == 0 and down:
                g = gu[slot, 0] + gu[slot, 1]
                act.append(g * jax.nn.sigmoid(g) * (gu[slot, 2] + gu[slot, 3]))
            if piece < 4:
                w_ref, k0 = (wg, wu)[piece // 2], piece % 2 * half
                cols = pl.ds(pl.multiple_of(jnp.minimum(t, n_ffn - 1) * LANES, LANES), LANES)
                gu[slot, piece] = _dot(xsel[:, k0:k0 + half], w_ref[k0 // 2:(k0 + half) // 2, cols])
            elif down:
                c0 = piece % 2 * half
                rows = pl.ds(pl.multiple_of((t - UNROLL) * (LANES // 2), LANES // 2), LANES // 2)
                yacc[:, c0:c0 + half] += _dot(act[0], wd[rows, c0:c0 + half])

        parts = []
        for i in range(H + n_col):
            if i < H:
                project(i)
            else:
                if i == H and first:
                    cp_wo.wait()
                    _start(cp_x_late)
                parts.append(out_proj(0, h_split, i - H, i - H + 1))
            if ffn_slice is not None and i - H in FFN_AFTER_TILE:
                ffn_piece(FFN_AFTER_TILE.index(i - H))
            if 0 <= i - lag_scores < H:
                scores(i - lag_scores)
            if 0 <= i - lag_mix < H:
                mix(i - lag_mix)
        assert h_split + lag_mix <= H and not qkv
        hi = jnp.concatenate(parts[c_split:], axis=1) + out_proj(h_split, H, c_split, n_col)
        lo = jnp.concatenate(parts[:c_split], axis=1) + out_proj(h_split, H, 0, c_split)
        o = jnp.concatenate([lo, hi], axis=1)

        if not last:
            hall[s + 1, :M, :] = o[:M]
        outbuf[s] = (xbuf[s].astype(F32) + o[M - q0:] + hall[s, M:, :]).astype(BF16)

    s_ffn, s_last = half_seg, n_seg - 2
    assert s_last - s_ffn == n_ffn + UNROLL and (s_ffn - 2) % UNROLL == 0 and n_ffn % UNROLL == 0

    step(0, ORDER_PLAIN, first=True)
    finish_segments([1])
    step(1, ORDER_PLAIN)
    finish_segments([2, half_seg + 1])
    _wait(cp_x_late)
    _start(cp_ffn)

    def norm_steps(j, carry):
        for u in range(UNROLL):
            s = 2 + UNROLL * j + u
            step(s, ORDER_PLAIN)
            finish_segments([s + 1, s + half_seg])
        return carry

    lax.fori_loop(0, (s_ffn - 2) // UNROLL, norm_steps, 0)

    _wait(cp_ffn)
    idx, gate = route()
    for u in range(UNROLL):
        step(s_ffn + u, ORDER_FFN, ffn_slice=(u, u, False))

    def ffn_steps(j, carry):
        for u in range(UNROLL):
            step(s_ffn + UNROLL * j + u, ORDER_FFN, ffn_slice=(UNROLL * j + u, u, True))
        return carry

    lax.fori_loop(1, (s_last - s_ffn) // UNROLL, ffn_steps, 0)

    def write_out(s0, s1, sem):
        row = lax.broadcasted_iota(jnp.int32, (T, D), 0)
        for n, i in enumerate(idx):
            @pl.when((i >= s0 * T) & (i < s1 * T))
            def _():
                blk = outbuf[i // T].astype(F32)
                upd = yacc[n:n + 1, :] * gate[n]
                outbuf[i // T] = jnp.where(row == i % T, blk + upd, blk).astype(BF16)
        cp = pltpu.make_async_copy(outbuf.at[s0:s1], out_hbm.at[s0:s1], sem)
        cp.start()
        return cp

    cp_head = write_out(0, s_last, sem_out.at[0])
    for s in range(s_last, n_seg):
        step(s, ORDER_PLAIN, last=s == n_seg - 1)
    _wait([cp_head, write_out(s_last, n_seg, sem_out.at[1])])


@functools.partial(jax.jit, static_argnames=("A_seg_len",))
def pallas_parallel_sum__memory_aug_recurrent_mem_tr__moe_arch_mod__prompt_kernel(
    A_x: jax.Array,
    A_mem0: jax.Array,
    A_Wq: jax.Array,
    A_Wk: jax.Array,
    A_Wv: jax.Array,
    A_Wo: jax.Array,
    A_seg_len: int,
    B_x: jax.Array,
    B_w_r: jax.Array,
    B_w_gate: jax.Array,
    B_w_up: jax.Array,
    B_w_down: jax.Array,
):
    del B_x
    B, S, D = A_x.shape
    _, H, Dh = A_Wq.shape
    M = A_mem0.shape[1]
    T = int(A_seg_len)
    F = B_w_gate.shape[1]
    L = M + T
    n_seg = S // T
    assert B == 1 and S % T == 0 and T % 16 == 0 and M % 8 == 0 and Dh == LANES and H % 2 == 0
    assert n_seg <= LANES

    any_spec = pl.BlockSpec(memory_space=pl.ANY)
    out = pl.pallas_call(
        _kernel,
        out_shape=jax.ShapeDtypeStruct((n_seg, T, D), A_x.dtype),
        in_specs=[any_spec] * 10,
        out_specs=any_spec,
        scratch_shapes=[
            pltpu.VMEM((n_seg, T, D), BF16),
            pltpu.VMEM((M, D), BF16),
            pltpu.VMEM((D,), BF16),
            pltpu.VMEM((n_seg, L, D), F32),
            pltpu.VMEM((H, D // 2, Dh), U32),
            pltpu.VMEM((H, D // 2, Dh), U32),
            pltpu.VMEM((H, D // 2, Dh), U32),
            pltpu.VMEM((H * Dh // 2, D), U32),
            pltpu.VMEM((H, n_seg * PRE, Dh), F32),
            pltpu.VMEM((H, n_seg * PRE, Dh), F32),
            pltpu.VMEM((2 * len(V_EARLY), n_seg * PRE, Dh), F32),
            pltpu.VMEM((5, n_seg * PRE // 2, D // 2), F32),
            pltpu.VMEM((L, H * Dh), F32),
            pltpu.VMEM((n_seg, T, D), BF16),
            pltpu.VMEM((T, LANES), F32),
            pltpu.VMEM((D // 2, F), U32),
            pltpu.VMEM((D // 2, F), U32),
            pltpu.VMEM((F // 2, D), U32),
            pltpu.VMEM((8, D), F32),
            pltpu.VMEM((8, D), F32),
            pltpu.VMEM((UNROLL, 4, 8, LANES), F32),
            pltpu.SemaphoreType.DMA((9,)),
            pltpu.SemaphoreType.DMA((3 * H // 2,)),
            pltpu.SemaphoreType.DMA((3,)),
            pltpu.SemaphoreType.DMA((2,)),
        ],
        compiler_params=pltpu.CompilerParams(vmem_limit_bytes=120 * 1024 * 1024),
        name="rmt_mod_fused",
    )(
        A_x.reshape(n_seg, T, D),
        A_mem0.reshape(M, D),
        A_Wq.reshape(D // 2, 2, H, Dh),
        A_Wk.reshape(D // 2, 2, H, Dh),
        A_Wv.reshape(D // 2, 2, H, Dh),
        A_Wo.reshape(H * Dh, D),
        B_w_r,
        B_w_gate,
        B_w_up,
        B_w_down,
    )
    return out.reshape(B, S, D)
```
